```python
import jax
import jax.numpy as jnp

def _softmax(x, axis=-1):
    return jax.nn.softmax(x, axis=axis)

def _gelu(x):
    return jax.nn.gelu(x, approximate=True)

def _silu(x):
    return jax.nn.silu(x)

def _sigmoid(x):
    return jax.nn.sigmoid(x)

def _layernorm(x, axis=-1, eps=1e-05):
    m = jnp.mean(x, axis=axis, keepdims=True)
    v = jnp.var(x, axis=axis, keepdims=True)
    return (x - m) / jnp.sqrt(v + eps)

def _scatter_add(tgt, idx, src, axis=0):
    return tgt.at[idx].add(src)

def _segment_sum(src, seg, n):
    return jax.ops.segment_sum(src, seg, n)

class _Rng:

    def __init__(self, key):
        self._k = key

    def _next(self):
        self._k, sub = jax.random.split(self._k)
        return sub

    def normal(self, shape):
        return jax.random.normal(self._next(), shape, dtype=jnp.bfloat16)

    def randint(self, lo, hi, shape):
        return jax.random.randint(self._next(), shape, lo, hi, dtype=jnp.int32)

    def uniform(self, shape, lo=0.0, hi=1.0):
        return jax.random.uniform(self._next(), shape, jnp.bfloat16, lo, hi)

    def permutation(self, n):
        return jax.random.permutation(self._next(), n)
kernel_name = 'standalone__autoregressive_conv_wavernn__speech'

def setup_inputs():
    _rng = _Rng(jax.random.key(int.from_bytes(__import__("os").urandom(4), "little")))
    _w = lambda a: (lambda t: t.astype(jnp.bfloat16) if jnp.issubdtype(t.dtype, jnp.floating) else t)(jnp.asarray(a))
    B, T, D, K = (2, 16000, 256, 31)
    return {'x': _w((lambda *s: _rng.normal(s) * 0.05)(B, T, D)), 'w': _w((lambda *s: _rng.normal(s) * 0.05)(K, D, 2 * D))}

def reference(x, w):
    B, T, D = x.shape
    K = w.shape[0]
    dil = 2
    pad = (K - 1) * dil
    xp = jnp.pad(x, ((0, 0), (pad, 0), (0, 0)))
    h = jnp.einsum('btd,de->bte', xp[:, 0:T, :], w[0])
    for i in range(1, K):
        h = h + jnp.einsum('btd,de->bte', xp[:, i * dil:i * dil + T, :], w[i])
    f, g = (h[..., :D].copy(), h[..., D:].copy())
    return jnp.tanh(f) * _sigmoid(g)
```

```python
import functools

import jax
import jax.numpy as jnp
import jax.experimental.pallas as pl
import jax.experimental.pallas.tpu as pltpu

_HALO = 64
_DIL = 2


def _kernel(xh_ref, xc_ref, w_ref, o_ref, xs_ref, *, tm, ktaps, d):
    t = pl.program_id(1)
    halo = xh_ref[...]
    xs_ref[0:_HALO, :] = jnp.where(t > 0, halo, jnp.zeros_like(halo))
    xs_ref[_HALO:, :] = xc_ref[...]
    first = _HALO - (ktaps - 1) * _DIL
    acc = None
    for i in range(ktaps):
        lhs = xs_ref[pl.ds(first + _DIL * i, tm), :]
        p = jnp.dot(lhs, w_ref[i], preferred_element_type=jnp.float32)
        acc = p if acc is None else acc + p
    f = acc[:, :d]
    g = acc[:, d:]
    o_ref[...] = (jnp.tanh(f) * jax.nn.sigmoid(g)).astype(o_ref.dtype)


@jax.jit
def pallas_standalone__autoregressive_conv_wavernn__speech_kernel(
    x: jax.Array,
    w: jax.Array,
):
    B, T, D = x.shape
    K = w.shape[0]
    tm = 640
    nt = T // tm
    hb = tm // _HALO
    return pl.pallas_call(
        functools.partial(_kernel, tm=tm, ktaps=K, d=D),
        grid=(B, nt),
        in_specs=[
            pl.BlockSpec((None, _HALO, D), lambda b, t: (b, jnp.maximum(t * hb - 1, 0), 0)),
            pl.BlockSpec((None, tm, D), lambda b, t: (b, t, 0)),
            pl.BlockSpec((K, D, 2 * D), lambda b, t: (0, 0, 0), pipeline_mode=pl.Buffered(1)),
        ],
        out_specs=pl.BlockSpec((None, tm, D), lambda b, t: (b, t, 0)),
        out_shape=jax.ShapeDtypeStruct((B, T, D), x.dtype),
        scratch_shapes=[pltpu.VMEM((_HALO + tm, D), x.dtype)],
        compiler_params=pltpu.CompilerParams(
            dimension_semantics=("arbitrary", "arbitrary"),
            vmem_limit_bytes=100 * 1024 * 1024),
    )(x, x, w)
```

```python
import functools
import math
import jax
import jax.numpy as jnp
import jax.experimental.pallas as pl
import jax.experimental.pallas.tpu as pltpu

HALO = 64
HALO32 = HALO // 2


class Node:
    def __init__(self, kind, parent, taps, nout, path):
        self.kind, self.parent, self.taps, self.nout, self.path = kind, parent, taps, nout, path
        self.depth = 0 if parent is None else parent.depth + 1
        self.children = None

    def din(self, r):
        k = self.kind
        if k == "K0": return [(1, 2 * r), (-1, 2 * r + 1)]
        if k == "Km": return [(1, 2 * r + 1)]
        if k == "K1": return [(1, 2 * r + 2), (-1, 2 * r + 1)]
        h = self.nout
        if k == "W0": return [(1, r), (-1, 2 * h + r)]
        if k == "W1": return [(1, h + r), (1, 2 * h + r)]
        if k == "W2": return [(1, 2 * h + r), (-1, h + r)]
        if k == "W3": return [(1, 3 * h + r), (-1, h + r)]
        raise ValueError(k)


def _tadd(a, b, sa=1.0, sb=1.0, scale=1.0):
    out = {}
    for d, s in ((a, sa), (b, sb)):
        for k, v in d.items():
            out[k] = out.get(k, 0.0) + s * v * scale
    return out


def build_tree(K, levels):
    nout = 1
    for lv in levels:
        nout *= 2 if lv == "K" else 3
    root = Node("root", None, [{k: 1.0} for k in range(K)], nout, ())
    def rec(n, rest):
        if not rest:
            return
        lv = rest[0]
        if lv == "K":
            h0, h1 = n.taps[0::2], n.taps[1::2]
            hs = [_tadd(h0[j], h1[j]) if j < len(h1) else h0[j] for j in range(len(h0))]
            n.children = [Node("K0", n, h0, n.nout // 2, n.path + (0,)), Node("Km", n, hs, n.nout // 2, n.path + (1,)),
                          Node("K1", n, h1, n.nout // 2, n.path + (2,))]
        else:
            h = n.nout // 3
            g0 = n.taps[:h]
            g1 = n.taps[h:]
            get = lambda j: g1[j] if j < len(g1) else {}
            n.children = [Node("W0", n, g0, h, n.path + (0,)),
                          Node("W1", n, [_tadd(g0[j], get(j), 1, 1, 0.5) for j in range(h)], h, n.path + (1,)),
                          Node("W2", n, [_tadd(g0[j], get(j), 1, -1, 0.5) for j in range(h)], h, n.path + (2,)),
                          Node("W3", n, g1, h, n.path + (3,))]
        for c in n.children:
            rec(c, rest[1:])
    rec(root, list(levels))
    return root


class Plan:
    def __init__(self, K, levels, mat, lead=1, cap_slack=1.15):
        self.root = build_tree(K, levels)
        self.P = self.root.nout
        self.mat = set(mat)
        self.leaf_seq = []
        self.arrays = 0
        self._solve_root()
        self._plan_prep(lead, cap_slack)

    def _new_arr(self):
        self.arrays += 1
        return self.arrays - 1

    def _solve(self, n, inits, sinks):
        if n.children is None:
            self.leaf_seq.append(("leaf", n, inits[0], sinks[0]))
            return
        c0, cm, c1 = n.children
        half = n.nout // 2
        mids = [self._new_arr() for _ in range(half)]
        self._solve(cm, [[] for _ in range(half)], [("store", m) for m in mids])
        self._solve(c0, [inits[2 * i] + [mids[i]] for i in range(half)], [sinks[2 * i] for i in range(half)])
        self._solve(c1, [inits[2 * i + 1] + [mids[i]] for i in range(half)], [sinks[2 * i + 1] for i in range(half)])

    def _solve_root(self):
        n = self.root
        P = self.P
        if n.children[0].kind == "K0":
            self._solve(n, [[] for _ in range(P)], [("final", p) for p in range(P)])
            return
        w0, w1, w2, w3 = n.children
        h = P // 3
        m1 = [self._new_arr() for _ in range(h)]
        s = [self._new_arr() for _ in range(h)]
        self._solve(w1, [[] for _ in range(h)], [("store", m) for m in m1])
        self._solve(w2, [[m1[i]] for i in range(h)], [("store", m) for m in s])
        n0 = len(self.leaf_seq)
        self._solve(w0, [[s[i]] for i in range(h)], [("final", i) for i in range(h)])
        n1 = len(self.leaf_seq)
        self._solve(w3, [[s[i]] for i in range(h)], [("final", 2 * h + i) for i in range(h)])
        n2 = len(self.leaf_seq)
        combs = [("comb", None, (m1[i], s[i]), ("final", h + i)) for i in range(h)]
        rest = self.leaf_seq[n0:]
        out = self.leaf_seq[:n0]
        every = max(1, len(rest) // (h + 1))
        ci = 0
        for i, it in enumerate(rest):
            out.append(it)
            if (i + 1) % every == 0 and ci < h:
                out.append(combs[ci]); ci += 1
        out += combs[ci:]
        self.leaf_seq = out

    def expr(self, n, r):
        if n.parent is None:
            return [(1, ("x", r))]
        terms = []
        for s, pr in n.din(r):
            for s2, src in self.resolve(n.parent, pr):
                terms.append((s * s2, src))
        return terms

    def resolve(self, n, r):
        if n.parent is None:
            return [(1, ("x", r))]
        if n.depth in self.mat:
            e = self.expr(n, r)
            if len(e) == 1 and e[0][0] == 1:
                return e
            key = ("a", n.path, r)
            self.prep_expr[key] = e
            return [(1, key)]
        return self.expr(n, r)

    def _plan_prep(self, lead, cap_slack):
        self.prep_expr = {}
        self.leaf_expr = {}
        first_use = {}
        items = self.leaf_seq
        for i, it in enumerate(items):
            if it[0] != "leaf":
                continue
            e = self.expr(it[1], 0)
            self.leaf_expr[it[1].path] = e
            for _, src in e:
                if src[0] == "a":
                    first_use.setdefault(src, i)
        depth_of = lambda key: len(key[1])
        tasks = sorted(self.prep_expr, key=lambda k: -depth_of(k))
        n = len(items)
        cap = max(1, math.ceil(len(tasks) / n * cap_slack))
        load = [0] * n
        slot = {}
        by_depth = {}
        for k in tasks:
            by_depth.setdefault(depth_of(k), []).append(k)
        deadline = dict(first_use)
        for d in sorted(by_depth, reverse=True):
            ks = sorted(by_depth[d], key=lambda k: -deadline[k])
            for k in ks:
                s = max(0, deadline[k] - lead)
                while s > 0 and load[s] >= cap:
                    s -= 1
                slot[k] = s
                load[s] += 1
                for _, src in self.prep_expr[k]:
                    if src[0] == "a":
                        deadline[src] = min(deadline.get(src, n), s)
        self.prep_at = [[] for _ in range(n)]
        for k in sorted(slot, key=lambda k: (slot[k], depth_of(k))):
            self.prep_at[slot[k]].append(k)
        ops = []
        for i, it in enumerate(items):
            for k in self.prep_at[i]:
                ops.append(("prep", k))
            ops.append(it)
        self.ops = ops
        last_use_in, last_use_out = {}, {}
        uses_out = {}
        for t, op in enumerate(ops):
            if op[0] == "prep":
                for _, src in self.prep_expr[op[1]]:
                    if src[0] == "a": last_use_in[src] = t
            elif op[0] == "leaf":
                for _, src in self.leaf_expr[op[1].path]:
                    if src[0] == "a": last_use_in[src] = t
                for a in op[2]: last_use_out[a] = t
            else:
                for a in op[2]: last_use_out[a] = t
        def alloc(defs, last):
            free, slots, nslots = [], {}, 0
            release = {}
            for k, t in last.items():
                release.setdefault(t, []).append(k)
            for t, k in defs:
                if k is not None:
                    if free: slots[k] = free.pop(0)
                    else: slots[k] = nslots; nslots += 1
                for r in release.get(t, []):
                    pending.append((t, r))
                while pending and pending[0][0] <= t - 2:
                    free.append(slots[pending.pop(0)[1]])
            return slots, nslots
        pending = []
        self.in_slot, self.n_in = alloc([(t, op[1] if op[0] == "prep" else None) for t, op in enumerate(ops)], last_use_in)
        pending = []
        self.out_slot, self.n_out = alloc(
            [(t, op[3][1] if op[0] in ("leaf", "comb") and op[3][0] == "store" else None) for t, op in enumerate(ops)], last_use_out)
        self.g_terms = []
        self.g_slot = {}
        for it in items:
            if it[0] == "leaf" and it[1].taps:
                assert len(it[1].taps) == 1
                self.g_slot[it[1].path] = len(self.g_terms)
                self.g_terms.append(it[1].taps[0])


def _pack(lo, hi):
    return pltpu.pack_elementwise([lo, hi], packed_dtype=jnp.bfloat16)


def _unpack(v):
    lo = pltpu.bitcast(v << 16, jnp.float32)
    hi = pltpu.bitcast(v & jnp.uint32(0xFFFF0000), jnp.float32)
    return lo, hi


def _signed_sum(terms):
    pos = [v for s, v in terms if s > 0]
    neg = [v for s, v in terms if s < 0]
    parts = []
    while pos and neg:
        parts.append(pos.pop(0) - neg.pop(0))
    parts += pos
    assert not neg or parts
    while len(parts) > 1:
        parts = [parts[i] + parts[i + 1] if i + 1 < len(parts) else parts[i] for i in range(0, len(parts), 2)]
    acc = parts[0]
    for v in neg:
        acc = acc - v
    return acc


def _kernel(xh_ref, xc_ref, w_ref, o_ref, pm_ref, g_ref, a_ref, b_ref, po_ref, *, plan, Q, K, D, opts):
    P = plan.P
    QS = Q + 4
    b = pl.program_id(0)
    t = pl.program_id(1)

    @pl.when(jnp.logical_and(b == 0, t == 0))
    def _():
        def body(i, carry):
            r0 = pl.multiple_of(i * 16, 16)
            s0 = pl.multiple_of(i * 8, 8)
            for nt in range(2 * D // 128):
                raw = {}
                def tap(k):
                    if k not in raw:
                        raw[k] = pltpu.bitcast(w_ref[k, pl.ds(r0, 16), nt * 128:(nt + 1) * 128], jnp.uint32)
                    return raw[k]
                memo = {}
                def gval(items):
                    if items in memo:
                        return memo[items]
                    if len(items) == 1:
                        k, cf = items[0]
                        lo, hi = _unpack(tap(k))
                        if cf != 1.0:
                            lo, hi = lo * cf, hi * cf
                    else:
                        m = len(items) // 2
                        (l0, h0), (l1, h1) = gval(items[:m]), gval(items[m:])
                        lo, hi = l0 + l1, h0 + h1
                    memo[items] = (lo, hi)
                    return lo, hi
                for s, terms in enumerate(plan.g_terms):
                    items = tuple(sorted(terms.items()))
                    if len(items) == 1 and items[0][1] == 1.0:
                        word = tap(items[0][0])
                    else:
                        lo, hi = gval(items)
                        word = _pack(lo, hi)
                    g_ref[s, nt, pl.ds(s0, 8), :] = word
            return carry
        jax.lax.fori_loop(0, D // 16, body, 0)

    pofs = P - HALO32
    for c in range(2):
        halo = pltpu.bitcast(xh_ref[:, c * 128:(c + 1) * 128], jnp.uint32)
        halo = jnp.where(t > 0, halo, jnp.zeros_like(halo))
        pm_ref[c, pl.ds(pofs * QS, HALO32, stride=QS), :] = halo
        for q in range(Q):
            v = pltpu.bitcast(xc_ref[pl.ds(2 * P * q, 2 * P), c * 128:(c + 1) * 128], jnp.uint32)
            pm_ref[c, pl.ds(q + 1, P, stride=QS), :] = v
    off0 = HALO32 - (K - 1) + pofs

    def load_src(src, c):
        if src[0] == "x":
            rho = src[1] + off0
            v = pm_ref[c, pl.ds((rho % P) * QS + rho // P, Q), :]
            return _unpack(v)
        sl = plan.in_slot[src]
        return a_ref[sl, c, 0], a_ref[sl, c, 1]

    def eval_expr(e, c):
        vals = [(s, load_src(src, c)) for s, src in e]
        lo = _signed_sum([(s, v[0]) for s, v in vals])
        hi = _signed_sum([(s, v[1]) for s, v in vals])
        return lo, hi

    def finish(y, p):
        o = (jnp.tanh(y[:, :D]) * jax.nn.sigmoid(y[:, D:])).astype(jnp.bfloat16)
        for c in range(2):
            po_ref[c, pl.ds(p * QS, Q), :] = pltpu.bitcast(o[:, c * 128:(c + 1) * 128], jnp.uint32)

    def sink(y, sk):
        if sk[0] == "final":
            finish(y, sk[1])
        else:
            b_ref[plan.out_slot[sk[1]]] = y

    for op in plan.ops:
        if op[0] == "prep":
            key = op[1]
            sl = plan.in_slot[key]
            for c in range(2):
                lo, hi = eval_expr(plan.prep_expr[key], c)
                a_ref[sl, c, 0] = lo
                a_ref[sl, c, 1] = hi
        elif op[0] == "leaf":
            _, n, inits, sk = op
            acc = None
            for a in inits:
                v = b_ref[plan.out_slot[a]]
                acc = v if acc is None else acc + v
            if n.taps:
                e = plan.leaf_expr[n.path]
                parts = []
                for c in range(2):
                    if len(e) == 1 and e[0][0] == 1 and e[0][1][0] == "x":
                        rho = e[0][1][1] + off0
                        word = pm_ref[c, pl.ds((rho % P) * QS + rho // P, Q), :]
                    else:
                        lo, hi = eval_expr(e, c)
                        word = _pack(lo, hi)
                    parts.append(pltpu.bitcast(word, jnp.bfloat16))
                lhs = jnp.concatenate(parts, axis=1)
                s = plan.g_slot[n.path]
                rhs = jnp.concatenate([pltpu.bitcast(g_ref[s, nt], jnp.bfloat16) for nt in range(2 * D // 128)], axis=1)
                pr = jnp.dot(lhs, rhs, preferred_element_type=jnp.float32)
                acc = pr if acc is None else acc + pr
            sink(acc, sk)
        else:
            _, _, (m1, s_), sk = op
            a1 = b_ref[plan.out_slot[m1]]
            y = a1 + (a1 - b_ref[plan.out_slot[s_]])
            sink(y, sk)

    for c in range(2):
        for q in range(Q):
            v = po_ref[c, pl.ds(q, P, stride=QS), :]
            o_ref[pl.ds(2 * P * q, 2 * P), c * 128:(c + 1) * 128] = pltpu.bitcast(v, jnp.bfloat16)


@jax.jit
def pallas_standalone__autoregressive_conv_wavernn__speech_kernel(
    x: jax.Array,
    w: jax.Array,
):
    levels, Q, mat, lead, slack, opts = "WKKKK", 24, (2, 3), 1, 1.15, {}
    B, T, D = x.shape
    K = w.shape[0]
    plan = Plan(K, levels, mat, lead, slack)
    P = plan.P
    TM = 2 * P * Q
    nt = pl.cdiv(T, TM)
    assert TM % HALO == 0
    hb = TM // HALO
    QS = Q + 4
    ng = len(plan.g_terms)
    return pl.pallas_call(
        functools.partial(_kernel, plan=plan, Q=Q, K=K, D=D, opts=opts),
        grid=(B, nt),
        in_specs=[
            pl.BlockSpec((None, HALO, D), lambda b, t: (b, jnp.maximum(t * hb - 1, 0), 0)),
            pl.BlockSpec((None, TM, D), lambda b, t: (b, t, 0)),
            pl.BlockSpec((K, D, 2 * D), lambda b, t: (0, 0, 0), pipeline_mode=pl.Buffered(1)),
        ],
        out_specs=pl.BlockSpec((None, TM, D), lambda b, t: (b, t, 0)),
        out_shape=jax.ShapeDtypeStruct((B, T, D), x.dtype),
        scratch_shapes=[
            pltpu.VMEM((2, P * QS + 8, 128), jnp.uint32),
            pltpu.VMEM((ng, 2 * D // 128, D // 2, 128), jnp.uint32),
            pltpu.VMEM((max(plan.n_in, 1), 2, 2, Q, 128), jnp.float32),
            pltpu.VMEM((max(plan.n_out, 1), 2 * Q, 2 * D), jnp.float32),
            pltpu.VMEM((2, P * QS, 128), jnp.uint32),
        ],
        compiler_params=pltpu.CompilerParams(
            dimension_semantics=("arbitrary", "arbitrary"),
            vmem_limit_bytes=124 * 1024 * 1024),
    )(x, x, w)
```

```python
import functools
import math
import jax
import jax.numpy as jnp
import jax.experimental.pallas as pl
import jax.experimental.pallas.tpu as pltpu

HALO = 64
HALO32 = HALO // 2


class Node:
    def __init__(self, kind, parent, taps, nout, path):
        self.kind, self.parent, self.taps, self.nout, self.path = kind, parent, taps, nout, path
        self.depth = 0 if parent is None else parent.depth + 1
        self.children = None

    def din(self, r):
        k = self.kind
        if k == "K0": return [(1, 2 * r), (-1, 2 * r + 1)]
        if k == "Km": return [(1, 2 * r + 1)]
        if k == "K1": return [(1, 2 * r + 2), (-1, 2 * r + 1)]
        h = self.nout
        if k == "B0": return [(1, r), (-1, h + r)]
        if k == "Bm": return [(1, h + r)]
        if k == "B1": return [(1, 2 * h + r), (-1, h + r)]
        if k == "W0": return [(1, r), (-1, 2 * h + r)]
        if k == "W1": return [(1, h + r), (1, 2 * h + r)]
        if k == "W2": return [(1, 2 * h + r), (-1, h + r)]
        if k == "W3": return [(1, 3 * h + r), (-1, h + r)]
        raise ValueError(k)


def _tadd(a, b, sa=1.0, sb=1.0, scale=1.0):
    out = {}
    for d, s in ((a, sa), (b, sb)):
        for k, v in d.items():
            out[k] = out.get(k, 0.0) + s * v * scale
    return out


def build_tree(K, levels):
    nout = 1
    for lv in levels:
        nout *= 2 if lv in "KB" else 3
    root = Node("root", None, [{k: 1.0} for k in range(K)], nout, ())
    def rec(n, rest):
        if not rest:
            return
        lv = rest[0]
        if lv == "K":
            h0, h1 = n.taps[0::2], n.taps[1::2]
            hs = [_tadd(h0[j], h1[j]) if j < len(h1) else h0[j] for j in range(len(h0))]
            n.children = [Node("K0", n, h0, n.nout // 2, n.path + (0,)), Node("Km", n, hs, n.nout // 2, n.path + (1,)),
                          Node("K1", n, h1, n.nout // 2, n.path + (2,))]
        elif lv == "B":
            h = n.nout // 2
            g0, g1 = n.taps[:h], n.taps[h:]
            gs = [_tadd(g0[j], g1[j]) if j < len(g1) else g0[j] for j in range(len(g0))]
            n.children = [Node("B0", n, g0, h, n.path + (0,)), Node("Bm", n, gs, h, n.path + (1,)),
                          Node("B1", n, g1, h, n.path + (2,))]
        else:
            h = n.nout // 3
            g0 = n.taps[:h]
            g1 = n.taps[h:]
            get = lambda j: g1[j] if j < len(g1) else {}
            n.children = [Node("W0", n, g0, h, n.path + (0,)),
                          Node("W1", n, [_tadd(g0[j], get(j), 1, 1, 0.5) for j in range(h)], h, n.path + (1,)),
                          Node("W2", n, [_tadd(g0[j], get(j), 1, -1, 0.5) for j in range(h)], h, n.path + (2,)),
                          Node("W3", n, g1, h, n.path + (3,))]
        for c in n.children:
            rec(c, rest[1:])
    rec(root, list(levels))
    return root


class Plan:
    def __init__(self, K, levels, mat, lead=1, cap_slack=1.15, Q=24, tail_len=36, unst=3, cap_add=0, xstage=True, xunst=True, head=True):
        self.root = build_tree(K, levels)
        self.P = self.root.nout
        self.mat = set(mat)
        self.leaf_seq = []
        self.arrays = 0
        self._solve_root()
        self.Q, self.tail_len, self.unst, self.cap_add = Q, tail_len, unst, cap_add
        self.xstage, self.xunst, self.use_head = xstage, xunst, head and xstage
        self._plan_prep(lead, cap_slack)

    def _new_arr(self):
        self.arrays += 1
        return self.arrays - 1

    def _solve(self, n, inits, sinks):
        if n.children is None:
            self.leaf_seq.append(("leaf", n, inits[0], sinks[0]))
            return
        c0, cm, c1 = n.children
        half = n.nout // 2
        mids = [self._new_arr() for _ in range(half)]
        self._solve(cm, [[] for _ in range(half)], [("store", m) for m in mids])
        if c0.kind == "B0":
            self._solve(c0, [inits[i] + [mids[i]] for i in range(half)], sinks[:half])
            self._solve(c1, [inits[half + i] + [mids[i]] for i in range(half)], sinks[half:])
            return
        self._solve(c0, [inits[2 * i] + [mids[i]] for i in range(half)], [sinks[2 * i] for i in range(half)])
        self._solve(c1, [inits[2 * i + 1] + [mids[i]] for i in range(half)], [sinks[2 * i + 1] for i in range(half)])

    def _solve_root(self):
        n = self.root
        P = self.P
        if n.children[0].kind in ("K0", "B0"):
            self._solve(n, [[] for _ in range(P)], [("final", p) for p in range(P)])
            return
        w0, w1, w2, w3 = n.children
        h = P // 3
        m1 = [self._new_arr() for _ in range(h)]
        s = [self._new_arr() for _ in range(h)]
        self._solve(w1, [[] for _ in range(h)], [("store", m) for m in m1])
        self._solve(w2, [[m1[i]] for i in range(h)], [("store", m) for m in s])
        n0 = len(self.leaf_seq)
        self._solve(w0, [[s[i]] for i in range(h)], [("final", i) for i in range(h)])
        n1 = len(self.leaf_seq)
        self._solve(w3, [[s[i]] for i in range(h)], [("final", 2 * h + i) for i in range(h)])
        n2 = len(self.leaf_seq)
        combs = [("comb", None, (m1[i], s[i]), ("final", h + i)) for i in range(h)]
        rest = self.leaf_seq[n0:]
        out = self.leaf_seq[:n0]
        every = max(1, len(rest) // (h + 1))
        ci = 0
        for i, it in enumerate(rest):
            out.append(it)
            if (i + 1) % every == 0 and ci < h:
                out.append(combs[ci]); ci += 1
        out += combs[ci:]
        self.leaf_seq = out

    def expr(self, n, r):
        if n.parent is None:
            return [(1, ("x", r))]
        terms = []
        for s, pr in n.din(r):
            for s2, src in self.resolve(n.parent, pr):
                terms.append((s * s2, src))
        return terms

    def resolve(self, n, r):
        if n.parent is None:
            return [(1, ("x", r))]
        if n.depth in self.mat:
            e = self.expr(n, r)
            if len(e) == 1 and e[0][0] == 1:
                return e
            key = ("a", n.path, r)
            self.prep_expr[key] = e
            return [(1, key)]
        return self.expr(n, r)

    def _plan_prep(self, lead, cap_slack):
        self.prep_expr = {}
        self.leaf_expr = {}
        first_use = {}
        items = self.leaf_seq
        for i, it in enumerate(items):
            if it[0] != "leaf":
                continue
            e = self.expr(it[1], 0)
            self.leaf_expr[it[1].path] = e
            for _, src in e:
                if src[0] == "a":
                    first_use.setdefault(src, i)
        depth_of = lambda key: len(key[1])
        tasks = sorted(self.prep_expr, key=lambda k: -depth_of(k))
        n = len(items)
        cap = max(1, math.ceil(len(tasks) / n * cap_slack)) + self.cap_add
        load = {}
        slot = {}
        by_depth = {}
        for k in tasks:
            by_depth.setdefault(depth_of(k), []).append(k)
        deadline = dict(first_use)
        x_limit = n - self.tail_len if self.xstage else n
        for d in sorted(by_depth, reverse=True):
            ks = sorted(by_depth[d], key=lambda k: -deadline[k])
            for k in ks:
                s = deadline[k] - lead
                if any(src[0] == "x" for _, src in self.prep_expr[k]):
                    s = min(s, x_limit)
                while load.get(s, 0) >= cap and (self.use_head or s > 0):
                    s -= 1
                if not self.use_head:
                    s = max(s, 0)
                slot[k] = s
                load[s] = load.get(s, 0) + 1
                for _, src in self.prep_expr[k]:
                    if src[0] == "a":
                        deadline[src] = min(deadline.get(src, n), s)
        for it in items:
            if it[0] == "leaf":
                assert all(src[0] == "a" for _, src in self.leaf_expr[it[1].path])
        self.prep_at = [[] for _ in range(n)]
        self.head = []
        for k in sorted(slot, key=lambda k: (slot[k], depth_of(k))):
            (self.head if slot[k] < 0 else self.prep_at[slot[k]]).append(k)
        first_final = min(i for i, it in enumerate(items) if it[3][0] == "final")
        un = [("unstage", c, q) for q in range(self.Q) for c in range(2)]
        u0 = self.unst
        span = max(1, first_final - 8 - u0)
        un_at = [[] for _ in range(n)]
        for i, op in enumerate(un):
            if self.xunst:
                un_at[u0 + i * span // len(un)].append(op)
        nxt = [("halo", c, 0) for c in range(2)] + [("stage", c, q) for q in range(self.Q) for c in range(2)]
        n_stage = len(nxt)
        nxt += [("prep", k) for k in self.head]
        w = [1.0] * n_stage + [2.5] * len(self.head)
        tot = sum(w)
        nx_at = [[] for _ in range(n)]
        accw = 0.0
        for op, wi in zip(nxt, w):
            if self.xstage:
                nx_at[x_limit + 1 + int(accw / tot * (self.tail_len - 3))].append(op)
            accw += wi
        ops = []
        for i, it in enumerate(items):
            ops += [("prep", k) for k in self.prep_at[i]]
            ops += un_at[i] + nx_at[i]
            ops.append(it)
        self.ops = ([] if self.xstage else nxt) + ops + ([] if self.xunst else un)
        self.prologue = nxt if self.xstage else []
        last_use_in, last_use_out = {}, {}
        uses_out = {}
        for t, op in enumerate(ops):
            if op[0] == "prep":
                for _, src in self.prep_expr[op[1]]:
                    if src[0] == "a": last_use_in[src] = t
            elif op[0] == "leaf":
                for _, src in self.leaf_expr[op[1].path]:
                    if src[0] == "a": last_use_in[src] = t
                for a in op[2]: last_use_out[a] = t
            elif op[0] == "comb":
                for a in op[2]: last_use_out[a] = t
        headset = set(self.head)
        def alloc(defs, last):
            free, slots, nslots = [], {}, 0
            for k in self.head if last is last_use_in else ():
                slots[k] = nslots; nslots += 1
            release = {}
            for k, t in last.items():
                if k not in headset:
                    release.setdefault(t, []).append(k)
            for t, k in defs:
                if k is not None and k not in headset:
                    if free: slots[k] = free.pop(0)
                    else: slots[k] = nslots; nslots += 1
                for r in release.get(t, []):
                    pending.append((t, r))
                while pending and pending[0][0] <= t - 2:
                    free.append(slots[pending.pop(0)[1]])
            return slots, nslots
        pending = []
        self.in_slot, self.n_in = alloc([(t, op[1] if op[0] == "prep" else None) for t, op in enumerate(ops)], last_use_in)
        pending = []
        self.out_slot, self.n_out = alloc(
            [(t, op[3][1] if op[0] in ("leaf", "comb") and op[3][0] == "store" else None) for t, op in enumerate(ops)], last_use_out)
        self.g_terms = []
        self.g_slot = {}
        for it in items:
            if it[0] == "leaf" and it[1].taps:
                assert len(it[1].taps) == 1
                self.g_slot[it[1].path] = len(self.g_terms)
                self.g_terms.append(it[1].taps[0])


def _pack(lo, hi):
    return pltpu.pack_elementwise([lo, hi], packed_dtype=jnp.bfloat16)


def _unpack(v):
    lo = pltpu.bitcast(v << 16, jnp.float32)
    hi = pltpu.bitcast(v & jnp.uint32(0xFFFF0000), jnp.float32)
    return lo, hi


def _signed_sum(terms):
    pos = [v for s, v in terms if s > 0]
    neg = [v for s, v in terms if s < 0]
    parts = []
    while pos and neg:
        parts.append(pos.pop(0) - neg.pop(0))
    parts += pos
    assert not neg or parts
    while len(parts) > 1:
        parts = [parts[i] + parts[i + 1] if i + 1 < len(parts) else parts[i] for i in range(0, len(parts), 2)]
    acc = parts[0]
    for v in neg:
        acc = acc - v
    return acc


def _kernel(xh_ref, xc_ref, w_hbm, o_ref, pm_ref, g_ref, a_ref, b_ref, po_ref, w_ref, w_sem, *, plan, Q, K, D, opts):
    step = pl.program_id(0)
    NS = opts["ns"]
    nblk, nb = opts["nblk"], opts["nb"]
    N = nblk * nb
    RW = D // NS

    def gvals(n, load_tap, memo, j, scale):
        key = (n.path, j)
        if key in memo:
            return memo[key]
        def f32(v):
            return _unpack(v[1]) if v[0] == "w" else (v[1], v[2])
        k = n.kind
        par = n.parent
        if k == "root":
            out = ("w", load_tap(j))
        elif k in ("W0", "W3"):
            out = gvals(par, load_tap, memo, j if k == "W0" else n.nout + j, scale)
            if scale != 1.0:
                lo, hi = f32(out)
                out = ("f", lo * scale, hi * scale)
        elif k == "B0":
            out = gvals(par, load_tap, memo, j, scale)
        elif k == "B1":
            out = gvals(par, load_tap, memo, n.nout + j, scale)
        elif k == "Bm":
            a = gvals(par, load_tap, memo, j, scale)
            if n.nout + j < len(par.taps):
                (l0, h0), (l1, h1) = f32(a), f32(gvals(par, load_tap, memo, n.nout + j, scale))
                out = ("f", l0 + l1, h0 + h1)
            else:
                out = a
        elif k == "K0":
            out = gvals(par, load_tap, memo, 2 * j, scale)
        elif k == "K1":
            out = gvals(par, load_tap, memo, 2 * j + 1, scale)
        elif k == "Km":
            a = gvals(par, load_tap, memo, 2 * j, scale)
            if 2 * j + 1 < len(par.taps):
                (l0, h0), (l1, h1) = f32(a), f32(gvals(par, load_tap, memo, 2 * j + 1, scale))
                out = ("f", l0 + l1, h0 + h1)
            else:
                out = a
        else:
            l0, h0 = f32(gvals(par, load_tap, memo, j, scale))
            if n.nout + j < len(par.taps):
                l1, h1 = f32(gvals(par, load_tap, memo, n.nout + j, scale))
                l0, h0 = (l0 + l1, h0 + h1) if k == "W1" else (l0 - l1, h0 - h1)
            out = ("f", l0 * (0.5 * scale), h0 * (0.5 * scale))
        memo[key] = out
        return out

    def g_leaves(n):
        if n.children is None:
            return [n] if n.taps else []
        order = n.children if n.children[0].kind == "W0" else (n.children[0], n.children[2], n.children[1])
        out = []
        for c in order:
            out += g_leaves(c)
        return out

    def w_copy(i):
        r = pl.ds(pl.multiple_of(i * RW, RW), RW)
        return pltpu.make_async_copy(w_hbm.at[:, r, :], w_ref.at[:, r, :], w_sem.at[i])

    def weight_transform():
        for i in range(NS):
            w_copy(i).start()

        def slab(i, carry):
            w_copy(i).wait()

            def body(ii, carry2):
                row = i * RW + ii * 16
                r0 = pl.multiple_of(row, 16)
                s0 = pl.multiple_of(row // 2, 8)
                for nt in range(2 * D // 128):
                    scale = 0.5 if nt >= D // 128 else 1.0
                    memo, top = {}, None
                    for lf in g_leaves(plan.root):
                        if lf.path[0] != top:
                            top, memo = lf.path[0], {}
                        def load_tap(k):
                            return pltpu.bitcast(w_ref[k, pl.ds(r0, 16), nt * 128:(nt + 1) * 128], jnp.uint32)
                        v = gvals(lf, load_tap, memo, 0, scale)
                        g_ref[plan.g_slot[lf.path], nt, pl.ds(s0, 8), :] = v[1] if v[0] == "w" else _pack(v[1], v[2])
                return carry2
            return jax.lax.fori_loop(0, RW // 16, body, carry)
        jax.lax.fori_loop(0, NS, slab, 0)

    P = plan.P
    QS = Q + 4
    pofs = P - HALO32
    off0 = HALO32 - (K - 1) + pofs

    def load_src(src, c):
        if src[0] == "x":
            rho = src[1] + off0
            return _unpack(pm_ref[c, pl.ds((rho % P) * QS + rho // P, Q), :])
        sl = plan.in_slot[src]
        return a_ref[sl, c, 0], a_ref[sl, c, 1]

    def eval_expr(e, c):
        vals = [(s, load_src(src, c)) for s, src in e]
        lo = _signed_sum([(s, v[0]) for s, v in vals])
        hi = _signed_sum([(s, v[1]) for s, v in vals])
        return lo, hi

    def finish(y, p):
        tf = jnp.tanh(y[:, :D])
        o = (0.5 * (tf * jnp.tanh(y[:, D:]) + tf)).astype(jnp.bfloat16)
        for c in range(2):
            po_ref[c, pl.ds(p * QS, Q), :] = pltpu.bitcast(o[:, c * 128:(c + 1) * 128], jnp.uint32)

    def sink(y, sk):
        if sk[0] == "final":
            finish(y, sk[1])
        else:
            b_ref[plan.out_slot[sk[1]]] = y

    def emit(ops, keep_halo):
        for op in ops:
            kind = op[0]
            if kind == "prep":
                key = op[1]
                sl = plan.in_slot[key]
                for c in range(2):
                    lo, hi = eval_expr(plan.prep_expr[key], c)
                    a_ref[sl, c, 0] = lo
                    a_ref[sl, c, 1] = hi
            elif kind == "leaf":
                _, n, inits, sk = op
                acc = None
                for a in inits:
                    v = b_ref[plan.out_slot[a]]
                    acc = v if acc is None else acc + v
                if n.taps:
                    e = plan.leaf_expr[n.path]
                    parts = []
                    for c in range(2):
                        lo, hi = eval_expr(e, c)
                        parts.append(pltpu.bitcast(_pack(lo, hi), jnp.bfloat16))
                    lhs = jnp.concatenate(parts, axis=1)
                    s = plan.g_slot[n.path]
                    rhs = jnp.concatenate([pltpu.bitcast(g_ref[s, nt], jnp.bfloat16) for nt in range(2 * D // 128)], axis=1)
                    pr = jnp.dot(lhs, rhs, preferred_element_type=jnp.float32)
                    acc = pr if acc is None else acc + pr
                sink(acc, sk)
            elif kind == "comb":
                _, _, (m1, s_), sk = op
                a1 = b_ref[plan.out_slot[m1]]
                sink(a1 + (a1 - b_ref[plan.out_slot[s_]]), sk)
            elif kind == "halo":
                c = op[1]
                halo = pltpu.bitcast(xh_ref[:, c * 128:(c + 1) * 128], jnp.uint32)
                pm_ref[c, pl.ds(pofs * QS, HALO32, stride=QS), :] = jnp.where(keep_halo, halo, jnp.zeros_like(halo))
            elif kind == "stage":
                _, c, q = op
                v = pltpu.bitcast(xc_ref[pl.ds(2 * P * q, 2 * P), c * 128:(c + 1) * 128], jnp.uint32)
                pm_ref[c, pl.ds(q + 1, P, stride=QS), :] = v
            else:
                _, c, q = op
                v = po_ref[c, pl.ds(q, P, stride=QS), :]
                o_ref[pl.ds(2 * P * q, 2 * P), c * 128:(c + 1) * 128] = pltpu.bitcast(v, jnp.bfloat16)

    @pl.when(step == 0)
    def _():
        weight_transform()
        if plan.xunst:
            po_ref[...] = jnp.zeros(po_ref.shape, po_ref.dtype)
        emit(plan.prologue, False)

    @pl.when(jnp.logical_and(step >= 1, step <= N))
    def _():
        o = 0 if plan.xstage else 1
        starts = step == nblk + o
        for i in range(2 if plan.xstage else 0, nb + 1):
            starts = jnp.logical_or(starts, step == i * nblk + o)
        emit(plan.ops, jnp.logical_not(starts))

    if plan.xunst:
        @pl.when(step == N + 1)
        def _():
            emit([("unstage", c, q) for q in range(Q) for c in range(2)], False)


@jax.jit
def pallas_standalone__autoregressive_conv_wavernn__speech_kernel(
    x: jax.Array,
    w: jax.Array,
):
    levels, Q, mat, lead, slack = "WKKKK", 24, (2, 3), 1, 1.15
    opts = dict(xstage=False, xunst=True, ns=16)
    B, T, D = x.shape
    K = w.shape[0]
    plan = Plan(K, levels, mat, lead, slack, Q, opts.get("tail_len", 36), opts.get("unst", 3), opts.get("cap_add", 0),
                opts.get("xstage", True), opts.get("xunst", True), opts.get("head", True))
    P = plan.P
    TM = 2 * P * Q
    nt = pl.cdiv(T, TM)
    assert TM % HALO == 0
    hb = TM // HALO
    QS = Q + 4
    ng = len(plan.g_terms)
    NS = opts.get("ns", 8)
    opts = dict(opts, ns=NS, nblk=nt, nb=B)
    N = B * nt

    def blk(i):
        b = sum((i >= k * nt).astype(jnp.int32) for k in range(1, B))
        return b, i - b * nt
    x_blk = lambda s: blk(jnp.minimum(s, N - 1) if plan.xstage else jnp.clip(s - 1, 0, N - 1))
    o_blk = lambda s: blk(jnp.maximum(s - 2, 0) if plan.xunst else jnp.clip(s - 1, 0, N - 1))
    return pl.pallas_call(
        functools.partial(_kernel, plan=plan, Q=Q, K=K, D=D, opts=opts),
        grid=(N + 2 if plan.xunst else N + 1,),
        in_specs=[
            pl.BlockSpec((None, HALO, D), lambda s: (x_blk(s)[0], jnp.maximum(x_blk(s)[1] * hb - 1, 0), 0)),
            pl.BlockSpec((None, TM, D), lambda s: (x_blk(s)[0], x_blk(s)[1], 0)),
            pl.BlockSpec(memory_space=pl.ANY),
        ],
        out_specs=pl.BlockSpec((None, TM, D), lambda s: (o_blk(s)[0], o_blk(s)[1], 0)),
        out_shape=jax.ShapeDtypeStruct((B, T, D), x.dtype),
        scratch_shapes=[
            pltpu.VMEM((2, P * QS + 8, 128), jnp.uint32),
            pltpu.VMEM((ng, 2 * D // 128, D // 2, 128), jnp.uint32),
            pltpu.VMEM((max(plan.n_in, 1), 2, 2, Q, 128), jnp.float32),
            pltpu.VMEM((max(plan.n_out, 1), 2 * Q, 2 * D), jnp.float32),
            pltpu.VMEM((2, P * QS, 128), jnp.uint32),
            pltpu.VMEM((K, D, 2 * D), w.dtype),
            pltpu.SemaphoreType.DMA((NS,)),
        ],
        compiler_params=pltpu.CompilerParams(
            dimension_semantics=("arbitrary",),
            vmem_limit_bytes=124 * 1024 * 1024),
    )(x, x, w)
```

```python
import functools
import math
import jax
import jax.numpy as jnp
import jax.experimental.pallas as pl
import jax.experimental.pallas.tpu as pltpu

HALO = 64
HALO32 = HALO // 2


class Node:
    def __init__(self, kind, parent, taps, nout, path):
        self.kind, self.parent, self.taps, self.nout, self.path = kind, parent, taps, nout, path
        self.depth = 0 if parent is None else parent.depth + 1
        self.children = None

    def din(self, r):
        k = self.kind
        if k == "K0": return [(1, 2 * r), (-1, 2 * r + 1)]
        if k == "Km": return [(1, 2 * r + 1)]
        if k == "K1": return [(1, 2 * r + 2), (-1, 2 * r + 1)]
        h = self.nout
        if k == "B0": return [(1, r), (-1, h + r)]
        if k == "Bm": return [(1, h + r)]
        if k == "B1": return [(1, 2 * h + r), (-1, h + r)]
        if k == "W0": return [(1, r), (-1, 2 * h + r)]
        if k == "W1": return [(1, h + r), (1, 2 * h + r)]
        if k == "W2": return [(1, 2 * h + r), (-1, h + r)]
        if k == "W3": return [(1, 3 * h + r), (-1, h + r)]
        raise ValueError(k)


def _tadd(a, b, sa=1.0, sb=1.0, scale=1.0):
    out = {}
    for d, s in ((a, sa), (b, sb)):
        for k, v in d.items():
            out[k] = out.get(k, 0.0) + s * v * scale
    return out


def build_tree(K, levels):
    nout = 1
    for lv in levels:
        nout *= 2 if lv in "KB" else 3
    root = Node("root", None, [{k: 1.0} for k in range(K)], nout, ())
    def rec(n, rest):
        if not rest:
            return
        lv = rest[0]
        if lv == "K":
            h0, h1 = n.taps[0::2], n.taps[1::2]
            hs = [_tadd(h0[j], h1[j]) if j < len(h1) else h0[j] for j in range(len(h0))]
            n.children = [Node("K0", n, h0, n.nout // 2, n.path + (0,)), Node("Km", n, hs, n.nout // 2, n.path + (1,)),
                          Node("K1", n, h1, n.nout // 2, n.path + (2,))]
        elif lv == "B":
            h = n.nout // 2
            g0, g1 = n.taps[:h], n.taps[h:]
            gs = [_tadd(g0[j], g1[j]) if j < len(g1) else g0[j] for j in range(len(g0))]
            n.children = [Node("B0", n, g0, h, n.path + (0,)), Node("Bm", n, gs, h, n.path + (1,)),
                          Node("B1", n, g1, h, n.path + (2,))]
        else:
            h = n.nout // 3
            g0 = n.taps[:h]
            g1 = n.taps[h:]
            get = lambda j: g1[j] if j < len(g1) else {}
            n.children = [Node("W0", n, g0, h, n.path + (0,)),
                          Node("W1", n, [_tadd(g0[j], get(j), 1, 1) for j in range(h)], h, n.path + (1,)),
                          Node("W2", n, [_tadd(g0[j], get(j), 1, -1) for j in range(h)], h, n.path + (2,)),
                          Node("W3", n, g1, h, n.path + (3,))]
        for c in n.children:
            rec(c, rest[1:])
    rec(root, list(levels))
    return root


class Plan:
    def __init__(self, K, levels, mat, lead=1, cap_slack=1.15, Q=24, tail_len=36, unst=3, cap_add=0, xstage=True, xunst=True, head=True, raw_ok=True):
        self.root = build_tree(K, levels)
        self.P = self.root.nout
        self.mat = set(mat)
        self.leaf_seq = []
        self.arrays = 0
        self._solve_root()
        self.Q, self.tail_len, self.unst, self.cap_add = Q, tail_len, unst, cap_add
        self.raw_ok = raw_ok
        self.xstage, self.xunst, self.use_head = xstage, xunst, head and xstage
        self._plan_prep(lead, cap_slack)

    def _new_arr(self):
        self.arrays += 1
        return self.arrays - 1

    def _solve(self, n, inits, sinks):
        if n.children is None:
            self.leaf_seq.append(("leaf", n, inits[0], sinks[0]))
            return
        c0, cm, c1 = n.children
        half = n.nout // 2
        mids = [self._new_arr() for _ in range(half)]
        self._solve(cm, [[] for _ in range(half)], [("store", m) for m in mids])
        if c0.kind == "B0":
            self._solve(c0, [inits[i] + [mids[i]] for i in range(half)], sinks[:half])
            self._solve(c1, [inits[half + i] + [mids[i]] for i in range(half)], sinks[half:])
            return
        self._solve(c0, [inits[2 * i] + [mids[i]] for i in range(half)], [sinks[2 * i] for i in range(half)])
        self._solve(c1, [inits[2 * i + 1] + [mids[i]] for i in range(half)], [sinks[2 * i + 1] for i in range(half)])

    def _solve_root(self):
        n = self.root
        P = self.P
        if n.children[0].kind in ("K0", "B0"):
            self._solve(n, [[] for _ in range(P)], [("final", p) for p in range(P)])
            return
        w0, w1, w2, w3 = n.children
        h = P // 3
        m1 = [self._new_arr() for _ in range(h)]
        s = [self._new_arr() for _ in range(h)]
        self._solve(w1, [[] for _ in range(h)], [("store", m) for m in m1])
        self._solve(w2, [[m1[i]] for i in range(h)], [("half", m) for m in s])
        n0 = len(self.leaf_seq)
        self._solve(w0, [[s[i]] for i in range(h)], [("final", i) for i in range(h)])
        n1 = len(self.leaf_seq)
        self._solve(w3, [[s[i]] for i in range(h)], [("final", 2 * h + i) for i in range(h)])
        n2 = len(self.leaf_seq)
        combs = [("comb", None, (m1[i], s[i]), ("final", h + i)) for i in range(h)]
        rest = self.leaf_seq[n0:]
        out = self.leaf_seq[:n0]
        every = max(1, len(rest) // (h + 1))
        ci = 0
        for i, it in enumerate(rest):
            out.append(it)
            if (i + 1) % every == 0 and ci < h:
                out.append(combs[ci]); ci += 1
        out += combs[ci:]
        self.leaf_seq = out

    def expr(self, n, r):
        if n.parent is None:
            return [(1, ("x", r))]
        terms = []
        for s, pr in n.din(r):
            for s2, src in self.resolve(n.parent, pr):
                terms.append((s * s2, src))
        return terms

    def resolve(self, n, r):
        if n.parent is None:
            return [(1, ("x", r))]
        if n.depth in self.mat:
            e = self.expr(n, r)
            if len(e) == 1 and e[0][0] == 1:
                return e
            key = ("a", n.path, r)
            self.prep_expr[key] = e
            return [(1, key)]
        return self.expr(n, r)

    def _plan_prep(self, lead, cap_slack):
        self.prep_expr = {}
        self.leaf_expr = {}
        first_use = {}
        items = self.leaf_seq
        for i, it in enumerate(items):
            if it[0] != "leaf":
                continue
            e = self.expr(it[1], 0)
            self.leaf_expr[it[1].path] = e
            for _, src in e:
                if src[0] == "a":
                    first_use.setdefault(src, i)
        depth_of = lambda key: len(key[1])
        tasks = sorted(self.prep_expr, key=lambda k: -depth_of(k))
        n = len(items)
        cap = max(1, math.ceil(len(tasks) / n * cap_slack)) + self.cap_add
        load = {}
        slot = {}
        by_depth = {}
        for k in tasks:
            by_depth.setdefault(depth_of(k), []).append(k)
        deadline = dict(first_use)
        x_limit = n - self.tail_len if self.xstage else n
        for d in sorted(by_depth, reverse=True):
            ks = sorted(by_depth[d], key=lambda k: -deadline[k])
            for k in ks:
                s = deadline[k] - lead
                if any(src[0] == "x" for _, src in self.prep_expr[k]):
                    s = min(s, x_limit)
                while load.get(s, 0) >= cap and (self.use_head or s > 0):
                    s -= 1
                if not self.use_head:
                    s = max(s, 0)
                slot[k] = s
                load[s] = load.get(s, 0) + 1
                for _, src in self.prep_expr[k]:
                    if src[0] == "a":
                        deadline[src] = min(deadline.get(src, n), s)
        for it in items:
            if it[0] == "leaf":
                assert all(src[0] == "a" for _, src in self.leaf_expr[it[1].path])
        self.prep_at = [[] for _ in range(n)]
        self.head = []
        for k in sorted(slot, key=lambda k: (slot[k], depth_of(k))):
            (self.head if slot[k] < 0 else self.prep_at[slot[k]]).append(k)
        first_final = min(i for i, it in enumerate(items) if it[3][0] == "final")
        un = [("unstage", c, q) for q in range(self.Q) for c in range(2)]
        u0 = self.unst
        span = max(1, first_final - 8 - u0)
        un_at = [[] for _ in range(n)]
        for i, op in enumerate(un):
            if self.xunst:
                un_at[u0 + i * span // len(un)].append(op)
        nxt = [("halo", c, 0) for c in range(2)] + [("stage", c, q) for q in range(self.Q) for c in range(2)]
        n_stage = len(nxt)
        nxt += [("prep", k) for k in self.head]
        w = [1.0] * n_stage + [2.5] * len(self.head)
        tot = sum(w)
        nx_at = [[] for _ in range(n)]
        accw = 0.0
        for op, wi in zip(nxt, w):
            if self.xstage:
                nx_at[x_limit + 1 + int(accw / tot * (self.tail_len - 3))].append(op)
            accw += wi
        ops = []
        for i, it in enumerate(items):
            ops += [("prep", k) for k in self.prep_at[i]]
            ops += un_at[i] + nx_at[i]
            ops.append(it)
        self.ops = ([] if self.xstage else nxt) + ops + ([] if self.xunst else un)
        self.prologue = nxt if self.xstage else []
        last_use_in, last_use_out = {}, {}
        uses_out = {}
        for t, op in enumerate(ops):
            if op[0] == "prep":
                for _, src in self.prep_expr[op[1]]:
                    if src[0] == "a": last_use_in[src] = t
            elif op[0] == "leaf":
                for _, src in self.leaf_expr[op[1].path]:
                    if src[0] == "a": last_use_in[src] = t
                for a in op[2]: last_use_out[a] = t
            elif op[0] == "comb":
                for a in op[2]: last_use_out[a] = t
        headset = set(self.head)
        def alloc(defs, last):
            free, slots, nslots = [], {}, 0
            for k in self.head if last is last_use_in else ():
                slots[k] = nslots; nslots += 1
            release = {}
            for k, t in last.items():
                if k not in headset:
                    release.setdefault(t, []).append(k)
            for t, k in defs:
                if k is not None and k not in headset:
                    if free: slots[k] = free.pop(0)
                    else: slots[k] = nslots; nslots += 1
                for r in release.get(t, []):
                    pending.append((t, r))
                while pending and pending[0][0] <= t - 2:
                    free.append(slots[pending.pop(0)[1]])
            return slots, nslots
        pending = []
        self.in_slot, self.n_in = alloc([(t, op[1] if op[0] == "prep" else None) for t, op in enumerate(ops)], last_use_in)
        pending = []
        self.out_slot, self.n_out = alloc(
            [(t, op[3][1] if op[0] in ("leaf", "comb") and op[3][0] in ("store", "half") else None) for t, op in enumerate(ops)], last_use_out)
        self.g_terms = []
        self.g_slot = {}
        self.g_raw = {}
        for it in items:
            if it[0] == "leaf" and it[1].taps:
                assert len(it[1].taps) == 1
                tp = it[1].taps[0]
                if self.raw_ok and it[1].path[0] in (0, 3) and len(tp) == 1:
                    self.g_raw[it[1].path] = next(iter(tp))
                    continue
                self.g_slot[it[1].path] = len(self.g_terms)
                self.g_terms.append(it[1].taps[0])


def _pack(lo, hi):
    return pltpu.pack_elementwise([lo, hi], packed_dtype=jnp.bfloat16)


def _unpack(v):
    lo = pltpu.bitcast(v << 16, jnp.float32)
    hi = pltpu.bitcast(v & jnp.uint32(0xFFFF0000), jnp.float32)
    return lo, hi


def _signed_sum(terms):
    pos = [v for s, v in terms if s > 0]
    neg = [v for s, v in terms if s < 0]
    parts = []
    while pos and neg:
        parts.append(pos.pop(0) - neg.pop(0))
    parts += pos
    assert not neg or parts
    while len(parts) > 1:
        parts = [parts[i] + parts[i + 1] if i + 1 < len(parts) else parts[i] for i in range(0, len(parts), 2)]
    acc = parts[0]
    for v in neg:
        acc = acc - v
    return acc


def _kernel(xh_ref, xc_ref, w_hbm, o_ref, pm_ref, g_ref, a_ref, b_ref, po_ref, w_ref, w_sem, *, plan, Q, K, D, opts):
    step = pl.program_id(0)
    NS = opts["ns"]
    nblk, nb = opts["nblk"], opts["nb"]
    N = nblk * nb
    RW = D // NS

    def gvals(n, load_tap, memo, j):
        key = (n.path, j)
        if key in memo:
            return memo[key]
        def f32(v):
            return _unpack(v[1]) if v[0] == "w" else (v[1], v[2])
        k = n.kind
        par = n.parent
        if k == "root":
            out = ("w", load_tap(j))
        elif k in ("W0", "W3"):
            out = gvals(par, load_tap, memo, j if k == "W0" else n.nout + j)
        elif k == "B0":
            out = gvals(par, load_tap, memo, j)
        elif k == "B1":
            out = gvals(par, load_tap, memo, n.nout + j)
        elif k == "Bm":
            a = gvals(par, load_tap, memo, j)
            if n.nout + j < len(par.taps):
                (l0, h0), (l1, h1) = f32(a), f32(gvals(par, load_tap, memo, n.nout + j))
                out = ("f", l0 + l1, h0 + h1)
            else:
                out = a
        elif k == "K0":
            out = gvals(par, load_tap, memo, 2 * j)
        elif k == "K1":
            out = gvals(par, load_tap, memo, 2 * j + 1)
        elif k == "Km":
            a = gvals(par, load_tap, memo, 2 * j)
            if 2 * j + 1 < len(par.taps):
                (l0, h0), (l1, h1) = f32(a), f32(gvals(par, load_tap, memo, 2 * j + 1))
                out = ("f", l0 + l1, h0 + h1)
            else:
                out = a
        else:
            l0, h0 = f32(gvals(par, load_tap, memo, j))
            if n.nout + j < len(par.taps):
                l1, h1 = f32(gvals(par, load_tap, memo, n.nout + j))
                l0, h0 = (l0 + l1, h0 + h1) if k == "W1" else (l0 - l1, h0 - h1)
            out = ("f", l0, h0)
        memo[key] = out
        return out

    def g_leaves(n):
        if n.children is None:
            return [n] if n.taps else []
        perm = opts.get("gtop", (0, 1, 2, 3)) if n.children[0].kind == "W0" else opts.get("gk", (0, 2, 1))
        order = [n.children[i] for i in perm]
        out = []
        for c in order:
            out += g_leaves(c)
        return out

    def w_copy(i):
        r = pl.ds(pl.multiple_of(i * RW, RW), RW)
        return pltpu.make_async_copy(w_hbm.at[:, r, :], w_ref.at[:, r, :], w_sem.at[i])

    def transform_rows(src_ref, row, dst_row):
        r0 = pl.multiple_of(row, 16)
        s0 = pl.multiple_of(dst_row // 2, 8)
        for nt in range(2 * D // 128):
            memo, top = {}, None
            for lf in g_leaves(plan.root):
                if lf.path not in plan.g_slot:
                    continue
                if lf.path[:opts.get("gscope", 1)] != top:
                    top, memo = lf.path[:opts.get("gscope", 1)], {}
                def load_tap(k):
                    return pltpu.bitcast(src_ref[k, pl.ds(r0, 16), nt * 128:(nt + 1) * 128], jnp.uint32)
                v = gvals(lf, load_tap, memo, 0)
                g_ref[plan.g_slot[lf.path], nt, pl.ds(s0, 8), :] = v[1] if v[0] == "w" else _pack(v[1], v[2])

    def weight_transform():
        for i in range(NS):
            w_copy(i).start()

        def slab(i, carry):
            w_copy(i).wait()

            def body(ii, carry2):
                row = i * RW + ii * 16
                transform_rows(w_ref, row, row)
                return carry2
            return jax.lax.fori_loop(0, RW // 16, body, carry)
        jax.lax.fori_loop(0, NS, slab, 0)

    P = plan.P
    QS = Q + 4
    pofs = P - HALO32
    off0 = HALO32 - (K - 1) + pofs

    def load_src(src, c):
        if src[0] == "x":
            rho = src[1] + off0
            return _unpack(pm_ref[c, pl.ds((rho % P) * QS + rho // P, Q), :])
        sl = plan.in_slot[src]
        return a_ref[sl, c, 0], a_ref[sl, c, 1]

    def eval_expr(e, c):
        vals = [(s, load_src(src, c)) for s, src in e]
        lo = _signed_sum([(s, v[0]) for s, v in vals])
        hi = _signed_sum([(s, v[1]) for s, v in vals])
        return lo, hi

    def finish(y, p):
        tf = jnp.tanh(y[:, :D])
        o = (0.5 * (tf * jnp.tanh(0.5 * y[:, D:]) + tf)).astype(jnp.bfloat16)
        for c in range(2):
            po_ref[c, pl.ds(p * QS, Q), :] = pltpu.bitcast(o[:, c * 128:(c + 1) * 128], jnp.uint32)

    def sink(y, sk):
        if sk[0] == "final":
            finish(y, sk[1])
        else:
            b_ref[plan.out_slot[sk[1]]] = y if sk[0] == "store" else 0.5 * y

    def emit(ops, keep_halo):
        for op in ops:
            kind = op[0]
            if kind == "prep":
                key = op[1]
                sl = plan.in_slot[key]
                for c in range(2):
                    lo, hi = eval_expr(plan.prep_expr[key], c)
                    a_ref[sl, c, 0] = lo
                    a_ref[sl, c, 1] = hi
            elif kind == "leaf":
                _, n, inits, sk = op
                acc = None
                for a in inits:
                    v = b_ref[plan.out_slot[a]]
                    acc = v if acc is None else acc + v
                if n.taps:
                    e = plan.leaf_expr[n.path]
                    parts = []
                    for c in range(2):
                        lo, hi = eval_expr(e, c)
                        parts.append(pltpu.bitcast(_pack(lo, hi), jnp.bfloat16))
                    lhs = jnp.concatenate(parts, axis=1)
                    if n.path in plan.g_raw:
                        rhs = w_ref[plan.g_raw[n.path]]
                    else:
                        s = plan.g_slot[n.path]
                        rhs = jnp.concatenate([pltpu.bitcast(g_ref[s, nt], jnp.bfloat16) for nt in range(2 * D // 128)], axis=1)
                    pr = jnp.dot(lhs, rhs, preferred_element_type=jnp.float32)
                    acc = pr if acc is None else acc + pr
                sink(acc, sk)
            elif kind == "comb":
                _, _, (m1, s_), sk = op
                sink(b_ref[plan.out_slot[m1]] - b_ref[plan.out_slot[s_]], sk)
            elif kind == "halo":
                c = op[1]
                halo = pltpu.bitcast(xh_ref[:, c * 128:(c + 1) * 128], jnp.uint32)
                pm_ref[c, pl.ds(pofs * QS, HALO32, stride=QS), :] = jnp.where(keep_halo, halo, jnp.zeros_like(halo))
            elif kind == "stage":
                _, c, q = op
                v = pltpu.bitcast(xc_ref[pl.ds(2 * P * q, 2 * P), c * 128:(c + 1) * 128], jnp.uint32)
                pm_ref[c, pl.ds(q + 1, P, stride=QS), :] = v
            else:
                _, c, q = op
                v = po_ref[c, pl.ds(q, P, stride=QS), :]
                o_ref[pl.ds(2 * P * q, 2 * P), c * 128:(c + 1) * 128] = pltpu.bitcast(v, jnp.bfloat16)

    @pl.when(step == 0)
    def _():
        weight_transform()
        if plan.xunst:
            po_ref[...] = jnp.zeros(po_ref.shape, po_ref.dtype)
        emit(plan.prologue, False)

    @pl.when(jnp.logical_and(step >= 1, step <= N))
    def _():
        o = 0 if plan.xstage else 1
        starts = step == nblk + o
        for i in range(2 if plan.xstage else 0, nb + 1):
            starts = jnp.logical_or(starts, step == i * nblk + o)
        emit(plan.ops, jnp.logical_not(starts))

    if plan.xunst:
        @pl.when(step == N + 1)
        def _():
            emit([("unstage", c, q) for q in range(Q) for c in range(2)], False)


@jax.jit
def pallas_standalone__autoregressive_conv_wavernn__speech_kernel(
    x: jax.Array,
    w: jax.Array,
):
    levels, Q, mat, lead, slack = "WBBKK", 24, (1, 2, 3), 1, 1.15
    opts = dict(xstage=False, xunst=True, ns=16, raw_ok=True, gtop=(1, 2, 0, 3), gscope=2)
    B, T, D = x.shape
    K = w.shape[0]
    plan = Plan(K, levels, mat, lead, slack, Q, opts.get("tail_len", 36), opts.get("unst", 3), opts.get("cap_add", 0),
                opts.get("xstage", True), opts.get("xunst", True), opts.get("head", True), opts.get("raw_ok", True))
    P = plan.P
    TM = 2 * P * Q
    nt = pl.cdiv(T, TM)
    assert TM % HALO == 0
    hb = TM // HALO
    QS = Q + 4
    ng = len(plan.g_terms)
    NS = opts.get("ns", 8)
    opts = dict(opts, ns=NS, nblk=nt, nb=B)
    N = B * nt

    def blk(i):
        b = sum((i >= k * nt).astype(jnp.int32) for k in range(1, B))
        return b, i - b * nt
    x_blk = lambda s: blk(jnp.minimum(s, N - 1) if plan.xstage else jnp.clip(s - 1, 0, N - 1))
    o_blk = lambda s: blk(jnp.maximum(s - 2, 0) if plan.xunst else jnp.clip(s - 1, 0, N - 1))
    return pl.pallas_call(
        functools.partial(_kernel, plan=plan, Q=Q, K=K, D=D, opts=opts),
        grid=(N + 2 if plan.xunst else N + 1,),
        in_specs=[
            pl.BlockSpec((None, HALO, D), lambda s: (x_blk(s)[0], jnp.maximum(x_blk(s)[1] * hb - 1, 0), 0)),
            pl.BlockSpec((None, TM, D), lambda s: (x_blk(s)[0], x_blk(s)[1], 0)),
            pl.BlockSpec(memory_space=pl.ANY),
        ],
        out_specs=pl.BlockSpec((None, TM, D), lambda s: (o_blk(s)[0], o_blk(s)[1], 0)),
        out_shape=jax.ShapeDtypeStruct((B, T, D), x.dtype),
        scratch_shapes=[
            pltpu.VMEM((2, P * QS + 8, 128), jnp.uint32),
            pltpu.VMEM((ng, 2 * D // 128, D // 2, 128), jnp.uint32),
            pltpu.VMEM((max(plan.n_in, 1), 2, 2, Q, 128), jnp.float32),
            pltpu.VMEM((max(plan.n_out, 1), 2 * Q, 2 * D), jnp.float32),
            pltpu.VMEM((2, P * QS, 128), jnp.uint32),
            pltpu.VMEM((K, D, 2 * D), w.dtype),
            pltpu.SemaphoreType.DMA((NS,)),
        ],
        compiler_params=pltpu.CompilerParams(
            dimension_semantics=("arbitrary",),
            vmem_limit_bytes=124 * 1024 * 1024),
    )(x, x, w)
```

```python
import functools
import math
import jax
import jax.numpy as jnp
import jax.experimental.pallas as pl
import jax.experimental.pallas.tpu as pltpu

HALO = 64
HALO32 = HALO // 2


class Node:
    def __init__(self, kind, parent, taps, nout, path):
        self.kind, self.parent, self.taps, self.nout, self.path = kind, parent, taps, nout, path
        self.depth = 0 if parent is None else parent.depth + 1
        self.children = None

    def din(self, r):
        k = self.kind
        if k == "K0": return [(1, 2 * r), (-1, 2 * r + 1)]
        if k == "Km": return [(1, 2 * r + 1)]
        if k == "K1": return [(1, 2 * r + 2), (-1, 2 * r + 1)]
        h = self.nout
        if k == "B0": return [(1, r), (-1, h + r)]
        if k == "Bm": return [(1, h + r)]
        if k == "B1": return [(1, 2 * h + r), (-1, h + r)]
        if k == "W0": return [(1, r), (-1, 2 * h + r)]
        if k == "W1": return [(1, h + r), (1, 2 * h + r)]
        if k == "W2": return [(1, 2 * h + r), (-1, h + r)]
        if k == "W3": return [(1, 3 * h + r), (-1, h + r)]
        raise ValueError(k)


def _tadd(a, b, sa=1.0, sb=1.0, scale=1.0):
    out = {}
    for d, s in ((a, sa), (b, sb)):
        for k, v in d.items():
            out[k] = out.get(k, 0.0) + s * v * scale
    return out


def build_tree(K, levels):
    nout = 1
    for lv in levels:
        nout *= 2 if lv in "KB" else 3
    root = Node("root", None, [{k: 1.0} for k in range(K)], nout, ())
    def rec(n, rest):
        if not rest:
            return
        lv = rest[0]
        if lv == "K":
            h0, h1 = n.taps[0::2], n.taps[1::2]
            hs = [_tadd(h0[j], h1[j]) if j < len(h1) else h0[j] for j in range(len(h0))]
            n.children = [Node("K0", n, h0, n.nout // 2, n.path + (0,)), Node("Km", n, hs, n.nout // 2, n.path + (1,)),
                          Node("K1", n, h1, n.nout // 2, n.path + (2,))]
        elif lv == "B":
            h = n.nout // 2
            g0, g1 = n.taps[:h], n.taps[h:]
            gs = [_tadd(g0[j], g1[j]) if j < len(g1) else g0[j] for j in range(len(g0))]
            n.children = [Node("B0", n, g0, h, n.path + (0,)), Node("Bm", n, gs, h, n.path + (1,)),
                          Node("B1", n, g1, h, n.path + (2,))]
        else:
            h = n.nout // 3
            g0 = n.taps[:h]
            g1 = n.taps[h:]
            get = lambda j: g1[j] if j < len(g1) else {}
            n.children = [Node("W0", n, g0, h, n.path + (0,)),
                          Node("W1", n, [_tadd(g0[j], get(j), 1, 1) for j in range(h)], h, n.path + (1,)),
                          Node("W2", n, [_tadd(g0[j], get(j), 1, -1) for j in range(h)], h, n.path + (2,)),
                          Node("W3", n, g1, h, n.path + (3,))]
        for c in n.children:
            rec(c, rest[1:])
    rec(root, list(levels))
    return root


class Plan:
    def __init__(self, K, levels, mat, lead=1, cap_slack=1.15, Q=24, tail_len=36, unst=3, cap_add=0, xstage=True, xunst=True, head=True, raw_ok=True):
        self.root = build_tree(K, levels)
        self.P = self.root.nout
        self.mat = set(mat)
        self.leaf_seq = []
        self.arrays = 0
        self._solve_root()
        self.Q, self.tail_len, self.unst, self.cap_add = Q, tail_len, unst, cap_add
        self.raw_ok = raw_ok
        self.xstage, self.xunst, self.use_head = xstage, xunst, head and xstage
        self._plan_prep(lead, cap_slack)

    def _new_arr(self):
        self.arrays += 1
        return self.arrays - 1

    def _solve(self, n, inits, sinks):
        if n.children is None:
            self.leaf_seq.append(("leaf", n, inits[0], sinks[0]))
            return
        c0, cm, c1 = n.children
        half = n.nout // 2
        mids = [self._new_arr() for _ in range(half)]
        self._solve(cm, [[] for _ in range(half)], [("store", m) for m in mids])
        if c0.kind == "B0":
            self._solve(c0, [inits[i] + [mids[i]] for i in range(half)], sinks[:half])
            self._solve(c1, [inits[half + i] + [mids[i]] for i in range(half)], sinks[half:])
            return
        self._solve(c0, [inits[2 * i] + [mids[i]] for i in range(half)], [sinks[2 * i] for i in range(half)])
        self._solve(c1, [inits[2 * i + 1] + [mids[i]] for i in range(half)], [sinks[2 * i + 1] for i in range(half)])

    def _solve_root(self):
        n = self.root
        P = self.P
        if n.children[0].kind in ("K0", "B0"):
            self._solve(n, [[] for _ in range(P)], [("final", p) for p in range(P)])
            return
        w0, w1, w2, w3 = n.children
        h = P // 3
        m1 = [self._new_arr() for _ in range(h)]
        s = [self._new_arr() for _ in range(h)]
        self._solve(w1, [[] for _ in range(h)], [("store", m) for m in m1])
        self._solve(w2, [[m1[i]] for i in range(h)], [("half", m) for m in s])
        n0 = len(self.leaf_seq)
        self._solve(w0, [[s[i]] for i in range(h)], [("final", i) for i in range(h)])
        n1 = len(self.leaf_seq)
        self._solve(w3, [[s[i]] for i in range(h)], [("final", 2 * h + i) for i in range(h)])
        n2 = len(self.leaf_seq)
        combs = [("comb", None, (m1[i], s[i]), ("final", h + i)) for i in range(h)]
        rest = self.leaf_seq[n0:]
        out = self.leaf_seq[:n0]
        every = max(1, len(rest) // (h + 1))
        ci = 0
        for i, it in enumerate(rest):
            out.append(it)
            if (i + 1) % every == 0 and ci < h:
                out.append(combs[ci]); ci += 1
        out += combs[ci:]
        self.leaf_seq = out

    def expr(self, n, r):
        if n.parent is None:
            return [(1, ("x", r))]
        terms = []
        for s, pr in n.din(r):
            for s2, src in self.resolve(n.parent, pr):
                terms.append((s * s2, src))
        return terms

    def resolve(self, n, r):
        if n.parent is None:
            return [(1, ("x", r))]
        if n.depth in self.mat:
            e = self.expr(n, r)
            if len(e) == 1 and e[0][0] == 1:
                return e
            key = ("a", n.path, r)
            self.prep_expr[key] = e
            return [(1, key)]
        return self.expr(n, r)

    def _plan_prep(self, lead, cap_slack):
        self.prep_expr = {}
        self.leaf_expr = {}
        first_use = {}
        items = self.leaf_seq
        for i, it in enumerate(items):
            if it[0] != "leaf":
                continue
            e = self.expr(it[1], 0)
            self.leaf_expr[it[1].path] = e
            for _, src in e:
                if src[0] == "a":
                    first_use.setdefault(src, i)
        depth_of = lambda key: len(key[1])
        tasks = sorted(self.prep_expr, key=lambda k: -depth_of(k))
        n = len(items)
        cap = max(1, math.ceil(len(tasks) / n * cap_slack)) + self.cap_add
        load = {}
        slot = {}
        by_depth = {}
        for k in tasks:
            by_depth.setdefault(depth_of(k), []).append(k)
        deadline = dict(first_use)
        x_limit = n - self.tail_len if self.xstage else n
        for d in sorted(by_depth, reverse=True):
            ks = sorted(by_depth[d], key=lambda k: -deadline[k])
            for k in ks:
                s = deadline[k] - lead
                if any(src[0] == "x" for _, src in self.prep_expr[k]):
                    s = min(s, x_limit)
                while load.get(s, 0) >= cap and (self.use_head or s > 0):
                    s -= 1
                if not self.use_head:
                    s = max(s, 0)
                slot[k] = s
                load[s] = load.get(s, 0) + 1
                for _, src in self.prep_expr[k]:
                    if src[0] == "a":
                        deadline[src] = min(deadline.get(src, n), s)
        for it in items:
            if it[0] == "leaf":
                assert all(src[0] == "a" for _, src in self.leaf_expr[it[1].path])
        self.prep_at = [[] for _ in range(n)]
        self.head = []
        for k in sorted(slot, key=lambda k: (slot[k], depth_of(k))):
            (self.head if slot[k] < 0 else self.prep_at[slot[k]]).append(k)
        first_final = min(i for i, it in enumerate(items) if it[3][0] == "final")
        un = [("unstage", c, q) for q in range(self.Q) for c in range(2)]
        u0 = self.unst
        span = max(1, first_final - 8 - u0)
        un_at = [[] for _ in range(n)]
        for i, op in enumerate(un):
            if self.xunst:
                un_at[u0 + i * span // len(un)].append(op)
        nxt = [("halo", c, 0) for c in range(2)] + [("stage", c, q) for q in range(self.Q) for c in range(2)]
        n_stage = len(nxt)
        nxt += [("prep", k) for k in self.head]
        w = [1.0] * n_stage + [2.5] * len(self.head)
        tot = sum(w)
        nx_at = [[] for _ in range(n)]
        accw = 0.0
        for op, wi in zip(nxt, w):
            if self.xstage:
                nx_at[x_limit + 1 + int(accw / tot * (self.tail_len - 3))].append(op)
            accw += wi
        ops = []
        for i, it in enumerate(items):
            ops += [("prep", k) for k in self.prep_at[i]]
            ops += un_at[i] + nx_at[i]
            ops.append(it)
        self.ops = ([] if self.xstage else nxt) + ops + ([] if self.xunst else un)
        self.prologue = nxt if self.xstage else []
        self.unstage_end = 1 + max(i for i, op in enumerate(self.ops) if op[0] == "unstage")
        last_use_in, last_use_out = {}, {}
        uses_out = {}
        for t, op in enumerate(ops):
            if op[0] == "prep":
                for _, src in self.prep_expr[op[1]]:
                    if src[0] == "a": last_use_in[src] = t
            elif op[0] == "leaf":
                for _, src in self.leaf_expr[op[1].path]:
                    if src[0] == "a": last_use_in[src] = t
                for a in op[2]: last_use_out[a] = t
            elif op[0] == "comb":
                for a in op[2]: last_use_out[a] = t
        headset = set(self.head)
        def alloc(defs, last):
            free, slots, nslots = [], {}, 0
            for k in self.head if last is last_use_in else ():
                slots[k] = nslots; nslots += 1
            release = {}
            for k, t in last.items():
                if k not in headset:
                    release.setdefault(t, []).append(k)
            for t, k in defs:
                if k is not None and k not in headset:
                    if free: slots[k] = free.pop(0)
                    else: slots[k] = nslots; nslots += 1
                for r in release.get(t, []):
                    pending.append((t, r))
                while pending and pending[0][0] <= t - 2:
                    free.append(slots[pending.pop(0)[1]])
            return slots, nslots
        pending = []
        self.in_slot, self.n_in = alloc([(t, op[1] if op[0] == "prep" else None) for t, op in enumerate(ops)], last_use_in)
        pending = []
        self.out_slot, self.n_out = alloc(
            [(t, op[3][1] if op[0] in ("leaf", "comb") and op[3][0] in ("store", "half") else None) for t, op in enumerate(ops)], last_use_out)
        self.g_terms = []
        self.g_slot = {}
        self.g_raw = {}
        for it in items:
            if it[0] == "leaf" and it[1].taps:
                assert len(it[1].taps) == 1
                tp = it[1].taps[0]
                if self.raw_ok and it[1].path[0] in (0, 3) and len(tp) == 1:
                    self.g_raw[it[1].path] = next(iter(tp))
                    continue
                self.g_slot[it[1].path] = len(self.g_terms)
                self.g_terms.append(it[1].taps[0])


def _pack(lo, hi):
    return pltpu.pack_elementwise([lo, hi], packed_dtype=jnp.bfloat16)


def _unpack(v):
    lo = pltpu.bitcast(v << 16, jnp.float32)
    hi = pltpu.bitcast(v & jnp.uint32(0xFFFF0000), jnp.float32)
    return lo, hi


def _signed_sum(terms):
    pos = [v for s, v in terms if s > 0]
    neg = [v for s, v in terms if s < 0]
    parts = []
    while pos and neg:
        parts.append(pos.pop(0) - neg.pop(0))
    parts += pos
    assert not neg or parts
    while len(parts) > 1:
        parts = [parts[i] + parts[i + 1] if i + 1 < len(parts) else parts[i] for i in range(0, len(parts), 2)]
    acc = parts[0]
    for v in neg:
        acc = acc - v
    return acc


def _kernel(x_hbm, w_hbm, o_hbm, pm_ref, g_ref, a_ref, b_ref, po_ref, w_ref, x_buf, o_buf, w_sem, x_sem, o_sem,
            *, plan, Q, K, D, T, opts):
    NS = opts["ns"]
    nblk, nb = opts["nblk"], opts["nb"]
    N = nblk * nb
    RW = D // NS
    TM = 2 * plan.P * Q

    def row0(t):
        return pl.multiple_of(jnp.where(t > 0, T - (nblk - t) * TM, 0), 16)

    def x_copies(b, t, slot):
        t0 = row0(t)
        h0 = pl.multiple_of(jnp.maximum(t0 - HALO, 0), 16)
        return (pltpu.make_async_copy(x_hbm.at[b, pl.ds(h0, HALO), :], x_buf.at[slot, pl.ds(0, HALO), :], x_sem.at[slot, 0]),
                pltpu.make_async_copy(x_hbm.at[b, pl.ds(t0, TM), :], x_buf.at[slot, pl.ds(HALO, TM), :], x_sem.at[slot, 1]))

    def o_copy(b, t, slot):
        return pltpu.make_async_copy(o_buf.at[slot], o_hbm.at[b, pl.ds(row0(t), TM), :], o_sem.at[slot])

    def gvals(n, load_tap, memo, j):
        key = (n.path, j)
        if key in memo:
            return memo[key]
        def f32(v):
            return _unpack(v[1]) if v[0] == "w" else (v[1], v[2])
        k = n.kind
        par = n.parent
        if k == "root":
            out = ("w", load_tap(j))
        elif k in ("W0", "W3"):
            out = gvals(par, load_tap, memo, j if k == "W0" else n.nout + j)
        elif k == "B0":
            out = gvals(par, load_tap, memo, j)
        elif k == "B1":
            out = gvals(par, load_tap, memo, n.nout + j)
        elif k == "Bm":
            a = gvals(par, load_tap, memo, j)
            if n.nout + j < len(par.taps):
                (l0, h0), (l1, h1) = f32(a), f32(gvals(par, load_tap, memo, n.nout + j))
                out = ("f", l0 + l1, h0 + h1)
            else:
                out = a
        elif k == "K0":
            out = gvals(par, load_tap, memo, 2 * j)
        elif k == "K1":
            out = gvals(par, load_tap, memo, 2 * j + 1)
        elif k == "Km":
            a = gvals(par, load_tap, memo, 2 * j)
            if 2 * j + 1 < len(par.taps):
                (l0, h0), (l1, h1) = f32(a), f32(gvals(par, load_tap, memo, 2 * j + 1))
                out = ("f", l0 + l1, h0 + h1)
            else:
                out = a
        else:
            l0, h0 = f32(gvals(par, load_tap, memo, j))
            if n.nout + j < len(par.taps):
                l1, h1 = f32(gvals(par, load_tap, memo, n.nout + j))
                l0, h0 = (l0 + l1, h0 + h1) if k == "W1" else (l0 - l1, h0 - h1)
            out = ("f", l0, h0)
        memo[key] = out
        return out

    def g_leaves(n):
        if n.children is None:
            return [n] if n.taps else []
        perm = opts.get("gtop", (0, 1, 2, 3)) if n.children[0].kind == "W0" else opts.get("gk", (0, 2, 1))
        order = [n.children[i] for i in perm]
        out = []
        for c in order:
            out += g_leaves(c)
        return out

    def w_copy(i):
        r = pl.ds(pl.multiple_of(i * RW, RW), RW)
        return pltpu.make_async_copy(w_hbm.at[:, r, :], w_ref.at[:, r, :], w_sem.at[i])

    def transform_rows(src_ref, row, dst_row):
        r0 = pl.multiple_of(row, 16)
        s0 = pl.multiple_of(dst_row // 2, 8)
        for nt in range(2 * D // 128):
            memo, top = {}, None
            for lf in g_leaves(plan.root):
                if lf.path not in plan.g_slot:
                    continue
                if lf.path[:opts.get("gscope", 1)] != top:
                    top, memo = lf.path[:opts.get("gscope", 1)], {}
                def load_tap(k):
                    return pltpu.bitcast(src_ref[k, pl.ds(r0, 16), nt * 128:(nt + 1) * 128], jnp.uint32)
                v = gvals(lf, load_tap, memo, 0)
                g_ref[plan.g_slot[lf.path], nt, pl.ds(s0, 8), :] = v[1] if v[0] == "w" else _pack(v[1], v[2])

    def weight_transform():
        def slab(i, carry):
            w_copy(i).wait()

            def body(ii, carry2):
                row = i * RW + ii * 16
                transform_rows(w_ref, row, row)
                return carry2
            return jax.lax.fori_loop(0, RW // 16, body, carry)
        jax.lax.fori_loop(0, NS, slab, 0)

    P = plan.P
    QS = Q + 4
    pofs = P - HALO32
    off0 = HALO32 - (K - 1) + pofs

    def load_src(src, c):
        if src[0] == "x":
            rho = src[1] + off0
            return _unpack(pm_ref[c, pl.ds((rho % P) * QS + rho // P, Q), :])
        sl = plan.in_slot[src]
        return a_ref[sl, c, 0], a_ref[sl, c, 1]

    def eval_expr(e, c):
        vals = [(s, load_src(src, c)) for s, src in e]
        lo = _signed_sum([(s, v[0]) for s, v in vals])
        hi = _signed_sum([(s, v[1]) for s, v in vals])
        return lo, hi

    def finish(y, p):
        tf = jnp.tanh(y[:, :D])
        o = (0.5 * (tf * jnp.tanh(0.5 * y[:, D:]) + tf)).astype(jnp.bfloat16)
        for c in range(2):
            po_ref[c, pl.ds(p * QS, Q), :] = pltpu.bitcast(o[:, c * 128:(c + 1) * 128], jnp.uint32)

    def sink(y, sk):
        if sk[0] == "final":
            finish(y, sk[1])
        else:
            b_ref[plan.out_slot[sk[1]]] = y if sk[0] == "store" else 0.5 * y

    def emit(ops, keep_halo, slot):
        for op in ops:
            kind = op[0]
            if kind == "prep":
                key = op[1]
                sl = plan.in_slot[key]
                for c in range(2):
                    lo, hi = eval_expr(plan.prep_expr[key], c)
                    a_ref[sl, c, 0] = lo
                    a_ref[sl, c, 1] = hi
            elif kind == "leaf":
                _, n, inits, sk = op
                acc = None
                for a in inits:
                    v = b_ref[plan.out_slot[a]]
                    acc = v if acc is None else acc + v
                if n.taps:
                    e = plan.leaf_expr[n.path]
                    parts = []
                    for c in range(2):
                        lo, hi = eval_expr(e, c)
                        parts.append(pltpu.bitcast(_pack(lo, hi), jnp.bfloat16))
                    lhs = jnp.concatenate(parts, axis=1)
                    if n.path in plan.g_raw:
                        rhs = w_ref[plan.g_raw[n.path]]
                    else:
                        s = plan.g_slot[n.path]
                        rhs = jnp.concatenate([pltpu.bitcast(g_ref[s, nt], jnp.bfloat16) for nt in range(2 * D // 128)], axis=1)
                    pr = jnp.dot(lhs, rhs, preferred_element_type=jnp.float32)
                    acc = pr if acc is None else acc + pr
                sink(acc, sk)
            elif kind == "comb":
                _, _, (m1, s_), sk = op
                sink(b_ref[plan.out_slot[m1]] - b_ref[plan.out_slot[s_]], sk)
            elif kind == "halo":
                c = op[1]
                halo = pltpu.bitcast(x_buf[slot, pl.ds(0, HALO), c * 128:(c + 1) * 128], jnp.uint32)
                pm_ref[c, pl.ds(pofs * QS, HALO32, stride=QS), :] = jnp.where(keep_halo, halo, jnp.zeros_like(halo))
            elif kind == "stage":
                _, c, q = op
                v = pltpu.bitcast(x_buf[slot, pl.ds(HALO + 2 * P * q, 2 * P), c * 128:(c + 1) * 128], jnp.uint32)
                pm_ref[c, pl.ds(q + 1, P, stride=QS), :] = v
            else:
                _, c, q = op
                v = po_ref[c, pl.ds(q, P, stride=QS), :]
                o_buf[slot, pl.ds(2 * P * q, 2 * P), c * 128:(c + 1) * 128] = pltpu.bitcast(v, jnp.bfloat16)

    zero = jnp.int32(0)
    for i in range(NS):
        w_copy(i).start()
    for cp in x_copies(zero, zero, 0):
        cp.start()
    po_ref[...] = jnp.zeros(po_ref.shape, po_ref.dtype)
    o_buf[1] = jnp.zeros(o_buf.shape[1:], o_buf.dtype)
    o_copy(zero, zero, 1).start()
    weight_transform()

    def step(n, carry):
        b, t, pb, pt = carry
        slot = n & 1
        last_t = t == nblk - 1
        is_last = n == N - 1
        nb_ = jnp.where(is_last, b, jnp.where(last_t, b + 1, b))
        nt_ = jnp.where(is_last, t, jnp.where(last_t, 0, t + 1))
        for cp in x_copies(b, t, slot):
            cp.wait()
        for cp in x_copies(nb_, nt_, 1 - slot):
            cp.start()
        emit(plan.ops, t > 0, slot)
        o_copy(pb, pt, 1 - slot).wait()
        o_copy(pb, pt, slot).start()
        return nb_, nt_, b, t

    b, t, pb, pt = jax.lax.fori_loop(0, N, step, (zero, zero, zero, zero))
    fs = N & 1
    emit([("unstage", c, q) for q in range(Q) for c in range(2)], False, fs)
    o_copy(pb, pt, fs).start()
    for cp in x_copies(b, t, fs):
        cp.wait()
    o_copy(pb, pt, 1 - fs).wait()
    o_copy(pb, pt, fs).wait()


@jax.jit
def pallas_standalone__autoregressive_conv_wavernn__speech_kernel(
    x: jax.Array,
    w: jax.Array,
):
    levels, Q, mat, lead, slack = "WBBKK", 24, (1, 2, 3), 1, 1.15
    opts = dict(xstage=False, xunst=True, ns=16, raw_ok=True, gtop=(1, 2, 0, 3), gscope=2)
    B, T, D = x.shape
    K = w.shape[0]
    plan = Plan(K, levels, mat, lead, slack, Q, opts.get("tail_len", 36), opts.get("unst", 3), opts.get("cap_add", 0),
                opts.get("xstage", True), opts.get("xunst", True), opts.get("head", True), opts.get("raw_ok", True))
    P = plan.P
    TM = 2 * P * Q
    nt = pl.cdiv(T, TM)
    assert TM % HALO == 0
    hb = TM // HALO
    QS = Q + 4
    ng = len(plan.g_terms)
    NS = opts.get("ns", 8)
    opts = dict(opts, ns=NS, nblk=nt, nb=B)
    N = B * nt

    assert not plan.xstage and plan.xunst and nt >= 3 and T % 16 == 0 and T - (nt - 1) * TM >= HALO
    return pl.pallas_call(
        functools.partial(_kernel, plan=plan, Q=Q, K=K, D=D, T=T, opts=opts),
        in_specs=[pl.BlockSpec(memory_space=pl.ANY), pl.BlockSpec(memory_space=pl.ANY)],
        out_specs=pl.BlockSpec(memory_space=pl.ANY),
        out_shape=jax.ShapeDtypeStruct((B, T, D), x.dtype),
        scratch_shapes=[
            pltpu.VMEM((2, P * QS + 8, 128), jnp.uint32),
            pltpu.VMEM((ng, 2 * D // 128, D // 2, 128), jnp.uint32),
            pltpu.VMEM((max(plan.n_in, 1), 2, 2, Q, 128), jnp.float32),
            pltpu.VMEM((max(plan.n_out, 1), 2 * Q, 2 * D), jnp.float32),
            pltpu.VMEM((2, P * QS, 128), jnp.uint32),
            pltpu.VMEM((K, D, 2 * D), w.dtype),
            pltpu.VMEM((2, HALO + TM, D), x.dtype),
            pltpu.VMEM((2, TM, D), x.dtype),
            pltpu.SemaphoreType.DMA((NS,)),
            pltpu.SemaphoreType.DMA((2, 2)),
            pltpu.SemaphoreType.DMA((2,)),
        ],
        compiler_params=pltpu.CompilerParams(
            vmem_limit_bytes=124 * 1024 * 1024),
    )(x, w)
```

```python
import functools
import math
import jax
import jax.numpy as jnp
import jax.experimental.pallas as pl
import jax.experimental.pallas.tpu as pltpu

HALO = 64
HALO32 = HALO // 2


class Node:
    def __init__(self, kind, parent, taps, nout, path):
        self.kind, self.parent, self.taps, self.nout, self.path = kind, parent, taps, nout, path
        self.depth = 0 if parent is None else parent.depth + 1
        self.children = None

    def din(self, r):
        k = self.kind
        if k == "K0": return [(1, 2 * r), (-1, 2 * r + 1)]
        if k == "Km": return [(1, 2 * r + 1)]
        if k == "K1": return [(1, 2 * r + 2), (-1, 2 * r + 1)]
        h = self.nout
        if k == "B0": return [(1, r), (-1, h + r)]
        if k == "Bm": return [(1, h + r)]
        if k == "B1": return [(1, 2 * h + r), (-1, h + r)]
        if k == "W0": return [(1, r), (-1, 2 * h + r)]
        if k == "W1": return [(1, h + r), (1, 2 * h + r)]
        if k == "W2": return [(1, 2 * h + r), (-1, h + r)]
        if k == "W3": return [(1, 3 * h + r), (-1, h + r)]
        raise ValueError(k)


def _tadd(a, b, sa=1.0, sb=1.0, scale=1.0):
    out = {}
    for d, s in ((a, sa), (b, sb)):
        for k, v in d.items():
            out[k] = out.get(k, 0.0) + s * v * scale
    return out


def build_tree(K, levels):
    nout = 1
    for lv in levels:
        nout *= 2 if lv in "KB" else 3
    root = Node("root", None, [{k: 1.0} for k in range(K)], nout, ())
    def rec(n, rest):
        if not rest:
            return
        lv = rest[0]
        if lv == "K":
            h0, h1 = n.taps[0::2], n.taps[1::2]
            hs = [_tadd(h0[j], h1[j]) if j < len(h1) else h0[j] for j in range(len(h0))]
            n.children = [Node("K0", n, h0, n.nout // 2, n.path + (0,)), Node("Km", n, hs, n.nout // 2, n.path + (1,)),
                          Node("K1", n, h1, n.nout // 2, n.path + (2,))]
        elif lv == "B":
            h = n.nout // 2
            g0, g1 = n.taps[:h], n.taps[h:]
            gs = [_tadd(g0[j], g1[j]) if j < len(g1) else g0[j] for j in range(len(g0))]
            n.children = [Node("B0", n, g0, h, n.path + (0,)), Node("Bm", n, gs, h, n.path + (1,)),
                          Node("B1", n, g1, h, n.path + (2,))]
        else:
            h = n.nout // 3
            g0 = n.taps[:h]
            g1 = n.taps[h:]
            get = lambda j: g1[j] if j < len(g1) else {}
            n.children = [Node("W0", n, g0, h, n.path + (0,)),
                          Node("W1", n, [_tadd(g0[j], get(j), 1, 1) for j in range(h)], h, n.path + (1,)),
                          Node("W2", n, [_tadd(g0[j], get(j), 1, -1) for j in range(h)], h, n.path + (2,)),
                          Node("W3", n, g1, h, n.path + (3,))]
        for c in n.children:
            rec(c, rest[1:])
    rec(root, list(levels))
    return root


class Plan:
    def __init__(self, K, levels, mat, lead=1, cap_slack=1.15, Q=24, tail_len=36, unst=3, cap_add=0, xstage=True, xunst=True, head=True, raw_ok=True):
        self.root = build_tree(K, levels)
        self.P = self.root.nout
        self.mat = set(mat)
        self.leaf_seq = []
        self.arrays = 0
        self._solve_root()
        self.Q, self.tail_len, self.unst, self.cap_add = Q, tail_len, unst, cap_add
        self.raw_ok = raw_ok
        self.xstage, self.xunst, self.use_head = xstage, xunst, head and xstage
        self._plan_prep(lead, cap_slack)

    def _new_arr(self):
        self.arrays += 1
        return self.arrays - 1

    def _solve(self, n, inits, sinks):
        if n.children is None:
            self.leaf_seq.append(("leaf", n, inits[0], sinks[0]))
            return
        c0, cm, c1 = n.children
        half = n.nout // 2
        mids = [self._new_arr() for _ in range(half)]
        self._solve(cm, [[] for _ in range(half)], [("store", m) for m in mids])
        if c0.kind == "B0":
            self._solve(c0, [inits[i] + [mids[i]] for i in range(half)], sinks[:half])
            self._solve(c1, [inits[half + i] + [mids[i]] for i in range(half)], sinks[half:])
            return
        self._solve(c0, [inits[2 * i] + [mids[i]] for i in range(half)], [sinks[2 * i] for i in range(half)])
        self._solve(c1, [inits[2 * i + 1] + [mids[i]] for i in range(half)], [sinks[2 * i + 1] for i in range(half)])

    def _solve_root(self):
        n = self.root
        P = self.P
        if n.children[0].kind in ("K0", "B0"):
            self._solve(n, [[] for _ in range(P)], [("final", p) for p in range(P)])
            return
        w0, w1, w2, w3 = n.children
        h = P // 3
        m1 = [self._new_arr() for _ in range(h)]
        s = [self._new_arr() for _ in range(h)]
        self._solve(w1, [[] for _ in range(h)], [("store", m) for m in m1])
        self._solve(w2, [[m1[i]] for i in range(h)], [("half", m) for m in s])
        n0 = len(self.leaf_seq)
        self._solve(w0, [[s[i]] for i in range(h)], [("final", i) for i in range(h)])
        n1 = len(self.leaf_seq)
        self._solve(w3, [[s[i]] for i in range(h)], [("final", 2 * h + i) for i in range(h)])
        n2 = len(self.leaf_seq)
        combs = [("comb", None, (m1[i], s[i]), ("final", h + i)) for i in range(h)]
        rest = self.leaf_seq[n0:]
        out = self.leaf_seq[:n0]
        every = max(1, len(rest) // (h + 1))
        ci = 0
        for i, it in enumerate(rest):
            out.append(it)
            if (i + 1) % every == 0 and ci < h:
                out.append(combs[ci]); ci += 1
        out += combs[ci:]
        self.leaf_seq = out

    def expr(self, n, r):
        if n.parent is None:
            return [(1, ("x", r))]
        terms = []
        for s, pr in n.din(r):
            for s2, src in self.resolve(n.parent, pr):
                terms.append((s * s2, src))
        return terms

    def resolve(self, n, r):
        if n.parent is None:
            return [(1, ("x", r))]
        if n.depth in self.mat:
            e = self.expr(n, r)
            if len(e) == 1 and e[0][0] == 1:
                return e
            key = ("a", n.path, r)
            self.prep_expr[key] = e
            return [(1, key)]
        return self.expr(n, r)

    def _plan_prep(self, lead, cap_slack):
        self.prep_expr = {}
        self.leaf_expr = {}
        first_use = {}
        items = self.leaf_seq
        for i, it in enumerate(items):
            if it[0] != "leaf":
                continue
            e = self.expr(it[1], 0)
            self.leaf_expr[it[1].path] = e
            for _, src in e:
                if src[0] == "a":
                    first_use.setdefault(src, i)
        depth_of = lambda key: len(key[1])
        tasks = sorted(self.prep_expr, key=lambda k: -depth_of(k))
        n = len(items)
        cap = max(1, math.ceil(len(tasks) / n * cap_slack)) + self.cap_add
        load = {}
        slot = {}
        by_depth = {}
        for k in tasks:
            by_depth.setdefault(depth_of(k), []).append(k)
        deadline = dict(first_use)
        x_limit = n - self.tail_len if self.xstage else n
        for d in sorted(by_depth, reverse=True):
            ks = sorted(by_depth[d], key=lambda k: -deadline[k])
            for k in ks:
                s = deadline[k] - lead
                if any(src[0] == "x" for _, src in self.prep_expr[k]):
                    s = min(s, x_limit)
                while load.get(s, 0) >= cap and (self.use_head or s > 0):
                    s -= 1
                if not self.use_head:
                    s = max(s, 0)
                slot[k] = s
                load[s] = load.get(s, 0) + 1
                for _, src in self.prep_expr[k]:
                    if src[0] == "a":
                        deadline[src] = min(deadline.get(src, n), s)
        for it in items:
            if it[0] == "leaf":
                assert all(src[0] == "a" for _, src in self.leaf_expr[it[1].path])
        self.prep_at = [[] for _ in range(n)]
        self.head = []
        for k in sorted(slot, key=lambda k: (slot[k], depth_of(k))):
            (self.head if slot[k] < 0 else self.prep_at[slot[k]]).append(k)
        first_final = min(i for i, it in enumerate(items) if it[3][0] == "final")
        un = [("unstage", c, q) for q in range(self.Q) for c in range(2)]
        u0 = self.unst
        span = max(1, first_final - 8 - u0)
        un_at = [[] for _ in range(n)]
        for i, op in enumerate(un):
            if self.xunst:
                un_at[u0 + i * span // len(un)].append(op)
        nxt = [("halo", c, 0) for c in range(2)] + [("stage", c, q) for q in range(self.Q) for c in range(2)]
        n_stage = len(nxt)
        nxt += [("prep", k) for k in self.head]
        w = [1.0] * n_stage + [2.5] * len(self.head)
        tot = sum(w)
        nx_at = [[] for _ in range(n)]
        accw = 0.0
        for op, wi in zip(nxt, w):
            if self.xstage:
                nx_at[x_limit + 1 + int(accw / tot * (self.tail_len - 3))].append(op)
            accw += wi
        ops = []
        for i, it in enumerate(items):
            ops += [("prep", k) for k in self.prep_at[i]]
            ops += un_at[i] + nx_at[i]
            ops.append(it)
        self.ops = ([] if self.xstage else nxt) + ops + ([] if self.xunst else un)
        self.prologue = nxt if self.xstage else []
        self.unstage_end = 1 + max(i for i, op in enumerate(self.ops) if op[0] == "unstage")
        last_use_in, last_use_out = {}, {}
        uses_out = {}
        for t, op in enumerate(ops):
            if op[0] == "prep":
                for _, src in self.prep_expr[op[1]]:
                    if src[0] == "a": last_use_in[src] = t
            elif op[0] == "leaf":
                for _, src in self.leaf_expr[op[1].path]:
                    if src[0] == "a": last_use_in[src] = t
                for a in op[2]: last_use_out[a] = t
            elif op[0] == "comb":
                for a in op[2]: last_use_out[a] = t
        headset = set(self.head)
        def alloc(defs, last):
            free, slots, nslots = [], {}, 0
            for k in self.head if last is last_use_in else ():
                slots[k] = nslots; nslots += 1
            release = {}
            for k, t in last.items():
                if k not in headset:
                    release.setdefault(t, []).append(k)
            for t, k in defs:
                if k is not None and k not in headset:
                    if free: slots[k] = free.pop(0)
                    else: slots[k] = nslots; nslots += 1
                for r in release.get(t, []):
                    pending.append((t, r))
                while pending and pending[0][0] <= t - 2:
                    free.append(slots[pending.pop(0)[1]])
            return slots, nslots
        pending = []
        self.in_slot, self.n_in = alloc([(t, op[1] if op[0] == "prep" else None) for t, op in enumerate(ops)], last_use_in)
        pending = []
        self.out_slot, self.n_out = alloc(
            [(t, op[3][1] if op[0] in ("leaf", "comb") and op[3][0] in ("store", "half") else None) for t, op in enumerate(ops)], last_use_out)
        self.g_terms = []
        self.g_slot = {}
        self.g_raw = {}
        for it in items:
            if it[0] == "leaf" and it[1].taps:
                assert len(it[1].taps) == 1
                tp = it[1].taps[0]
                if self.raw_ok and it[1].path[0] in (0, 3) and len(tp) == 1:
                    self.g_raw[it[1].path] = next(iter(tp))
                    continue
                self.g_slot[it[1].path] = len(self.g_terms)
                self.g_terms.append(it[1].taps[0])


def _pack(lo, hi):
    return pltpu.pack_elementwise([lo, hi], packed_dtype=jnp.bfloat16)


def _unpack(v):
    lo = pltpu.bitcast(v << 16, jnp.float32)
    hi = pltpu.bitcast(v & jnp.uint32(0xFFFF0000), jnp.float32)
    return lo, hi


def _signed_sum(terms):
    pos = [v for s, v in terms if s > 0]
    neg = [v for s, v in terms if s < 0]
    parts = []
    while pos and neg:
        parts.append(pos.pop(0) - neg.pop(0))
    parts += pos
    assert not neg or parts
    while len(parts) > 1:
        parts = [parts[i] + parts[i + 1] if i + 1 < len(parts) else parts[i] for i in range(0, len(parts), 2)]
    acc = parts[0]
    for v in neg:
        acc = acc - v
    return acc


def _kernel(x_hbm, w_hbm, o_hbm, pm_ref, g_ref, a_ref, b_ref, po_ref, w_ref, x_buf, o_buf, w_sem, x_sem, o_sem,
            *, plan, Q, K, D, T, opts):
    NS = opts["ns"]
    nblk, nb = opts["nblk"], opts["nb"]
    N = nblk * nb
    RW = D // NS
    TM = 2 * plan.P * Q

    def row0(t):
        return pl.multiple_of(jnp.where(t > 0, T - (nblk - t) * TM, 0), 16)

    def x_copies(b, t, slot):
        t0 = row0(t)
        h0 = pl.multiple_of(jnp.maximum(t0 - HALO, 0), 16)
        return (pltpu.make_async_copy(x_hbm.at[b, pl.ds(h0, HALO), :], x_buf.at[slot, pl.ds(0, HALO), :], x_sem.at[slot, 0]),
                pltpu.make_async_copy(x_hbm.at[b, pl.ds(t0, TM), :], x_buf.at[slot, pl.ds(HALO, TM), :], x_sem.at[slot, 1]))

    def o_copy(b, t, slot):
        return pltpu.make_async_copy(o_buf.at[slot], o_hbm.at[b, pl.ds(row0(t), TM), :], o_sem.at[slot])

    def gvals(n, load_tap, memo, j):
        key = (n.path, j)
        if key in memo:
            return memo[key]
        def f32(v):
            return _unpack(v[1]) if v[0] == "w" else (v[1], v[2])
        k = n.kind
        par = n.parent
        if k == "root":
            out = ("w", load_tap(j))
        elif k in ("W0", "W3"):
            out = gvals(par, load_tap, memo, j if k == "W0" else n.nout + j)
        elif k == "B0":
            out = gvals(par, load_tap, memo, j)
        elif k == "B1":
            out = gvals(par, load_tap, memo, n.nout + j)
        elif k == "Bm":
            a = gvals(par, load_tap, memo, j)
            if n.nout + j < len(par.taps):
                (l0, h0), (l1, h1) = f32(a), f32(gvals(par, load_tap, memo, n.nout + j))
                out = ("f", l0 + l1, h0 + h1)
            else:
                out = a
        elif k == "K0":
            out = gvals(par, load_tap, memo, 2 * j)
        elif k == "K1":
            out = gvals(par, load_tap, memo, 2 * j + 1)
        elif k == "Km":
            a = gvals(par, load_tap, memo, 2 * j)
            if 2 * j + 1 < len(par.taps):
                (l0, h0), (l1, h1) = f32(a), f32(gvals(par, load_tap, memo, 2 * j + 1))
                out = ("f", l0 + l1, h0 + h1)
            else:
                out = a
        else:
            l0, h0 = f32(gvals(par, load_tap, memo, j))
            if n.nout + j < len(par.taps):
                l1, h1 = f32(gvals(par, load_tap, memo, n.nout + j))
                l0, h0 = (l0 + l1, h0 + h1) if k == "W1" else (l0 - l1, h0 - h1)
            out = ("f", l0, h0)
        memo[key] = out
        return out

    def g_leaves(n):
        if n.children is None:
            return [n] if n.taps else []
        perm = opts.get("gtop", (0, 1, 2, 3)) if n.children[0].kind == "W0" else opts.get("gk", (0, 2, 1))
        order = [n.children[i] for i in perm]
        out = []
        for c in order:
            out += g_leaves(c)
        return out

    def w_copy(i):
        r = pl.ds(pl.multiple_of(i * RW, RW), RW)
        return pltpu.make_async_copy(w_hbm.at[:, r, :], w_ref.at[:, r, :], w_sem.at[i])

    def transform_rows(src_ref, row, dst_row):
        r0 = pl.multiple_of(row, 16)
        s0 = pl.multiple_of(dst_row // 2, 8)
        for nt in range(2 * D // 128):
            memo, top = {}, None
            for lf in g_leaves(plan.root):
                if lf.path not in plan.g_slot:
                    continue
                if lf.path[:opts.get("gscope", 1)] != top:
                    top, memo = lf.path[:opts.get("gscope", 1)], {}
                def load_tap(k):
                    return pltpu.bitcast(src_ref[k, pl.ds(r0, 16), nt * 128:(nt + 1) * 128], jnp.uint32)
                v = gvals(lf, load_tap, memo, 0)
                g_ref[plan.g_slot[lf.path], nt, pl.ds(s0, 8), :] = v[1] if v[0] == "w" else _pack(v[1], v[2])

    def weight_transform(start_rest):
        depth = opts.get("wdepth", 3)
        for i in range(depth):
            w_copy(i).start()
        po_ref[...] = jnp.zeros(po_ref.shape, po_ref.dtype)
        o_buf[1] = jnp.zeros(o_buf.shape[1:], o_buf.dtype)

        def slab(i, prefetch):
            w_copy(i).wait()
            if prefetch:
                w_copy(i + depth).start()

            def body(ii, carry2):
                row = i * RW + ii * 16
                transform_rows(w_ref, row, row)
                return carry2
            return jax.lax.fori_loop(0, RW // 16, body, 0)
        jax.lax.fori_loop(0, NS - depth, lambda i, c: slab(i, True), 0)
        start_rest()
        jax.lax.fori_loop(NS - depth, NS, lambda i, c: slab(i, False), 0)

    P = plan.P
    QS = Q + 4
    pofs = P - HALO32
    off0 = HALO32 - (K - 1) + pofs

    def load_src(src, c):
        if src[0] == "x":
            rho = src[1] + off0
            return _unpack(pm_ref[c, pl.ds((rho % P) * QS + rho // P, Q), :])
        sl = plan.in_slot[src]
        return a_ref[sl, c, 0], a_ref[sl, c, 1]

    def eval_expr(e, c):
        vals = [(s, load_src(src, c)) for s, src in e]
        lo = _signed_sum([(s, v[0]) for s, v in vals])
        hi = _signed_sum([(s, v[1]) for s, v in vals])
        return lo, hi

    def finish(y, p):
        tf = jnp.tanh(y[:, :D])
        o = (0.5 * (tf * jnp.tanh(0.5 * y[:, D:]) + tf)).astype(jnp.bfloat16)
        for c in range(2):
            po_ref[c, pl.ds(p * QS, Q), :] = pltpu.bitcast(o[:, c * 128:(c + 1) * 128], jnp.uint32)

    def sink(y, sk):
        if sk[0] == "final":
            finish(y, sk[1])
        else:
            b_ref[plan.out_slot[sk[1]]] = y if sk[0] == "store" else 0.5 * y

    def emit(ops, keep_halo, slot):
        for op in ops:
            kind = op[0]
            if kind == "prep":
                key = op[1]
                sl = plan.in_slot[key]
                for c in range(2):
                    lo, hi = eval_expr(plan.prep_expr[key], c)
                    a_ref[sl, c, 0] = lo
                    a_ref[sl, c, 1] = hi
            elif kind == "leaf":
                _, n, inits, sk = op
                acc = None
                for a in inits:
                    v = b_ref[plan.out_slot[a]]
                    acc = v if acc is None else acc + v
                if n.taps:
                    e = plan.leaf_expr[n.path]
                    parts = []
                    for c in range(2):
                        lo, hi = eval_expr(e, c)
                        parts.append(pltpu.bitcast(_pack(lo, hi), jnp.bfloat16))
                    lhs = jnp.concatenate(parts, axis=1)
                    if n.path in plan.g_raw:
                        rhs = w_ref[plan.g_raw[n.path]]
                    else:
                        s = plan.g_slot[n.path]
                        rhs = jnp.concatenate([pltpu.bitcast(g_ref[s, nt], jnp.bfloat16) for nt in range(2 * D // 128)], axis=1)
                    pr = jnp.dot(lhs, rhs, preferred_element_type=jnp.float32)
                    acc = pr if acc is None else acc + pr
                sink(acc, sk)
            elif kind == "comb":
                _, _, (m1, s_), sk = op
                sink(b_ref[plan.out_slot[m1]] - b_ref[plan.out_slot[s_]], sk)
            elif kind == "halo":
                c = op[1]
                halo = pltpu.bitcast(x_buf[slot, pl.ds(0, HALO), c * 128:(c + 1) * 128], jnp.uint32)
                pm_ref[c, pl.ds(pofs * QS, HALO32, stride=QS), :] = jnp.where(keep_halo, halo, jnp.zeros_like(halo))
            elif kind == "stage":
                _, c, q = op
                v = pltpu.bitcast(x_buf[slot, pl.ds(HALO + 2 * P * q, 2 * P), c * 128:(c + 1) * 128], jnp.uint32)
                pm_ref[c, pl.ds(q + 1, P, stride=QS), :] = v
            else:
                _, c, q = op
                v = po_ref[c, pl.ds(q, P, stride=QS), :]
                o_buf[slot, pl.ds(2 * P * q, 2 * P), c * 128:(c + 1) * 128] = pltpu.bitcast(v, jnp.bfloat16)

    zero = jnp.int32(0)
    def start_rest():
        for cp in x_copies(zero, zero, 0):
            cp.start()
        o_copy(zero, zero, 1).start()
    weight_transform(start_rest)

    def step(n, carry):
        b, t, pb, pt = carry
        slot = n & 1
        last_t = t == nblk - 1
        is_last = n == N - 1
        nb_ = jnp.where(is_last, b, jnp.where(last_t, b + 1, b))
        nt_ = jnp.where(is_last, t, jnp.where(last_t, 0, t + 1))
        for cp in x_copies(b, t, slot):
            cp.wait()
        for cp in x_copies(nb_, nt_, 1 - slot):
            cp.start()
        emit(plan.ops, t > 0, slot)
        o_copy(pb, pt, 1 - slot).wait()
        o_copy(pb, pt, slot).start()
        return nb_, nt_, b, t

    b, t, pb, pt = jax.lax.fori_loop(0, N, step, (zero, zero, zero, zero))
    fs = N & 1
    emit([("unstage", c, q) for q in range(Q) for c in range(2)], False, fs)
    o_copy(pb, pt, fs).start()
    for cp in x_copies(b, t, fs):
        cp.wait()
    o_copy(pb, pt, 1 - fs).wait()
    o_copy(pb, pt, fs).wait()


@jax.jit
def pallas_standalone__autoregressive_conv_wavernn__speech_kernel(
    x: jax.Array,
    w: jax.Array,
):
    levels, Q, mat, lead, slack = "WBBKK", 24, (1, 2, 3), 1, 1.15
    opts = dict(xstage=False, xunst=True, ns=16, raw_ok=True, gtop=(1, 2, 0, 3), gscope=2, wdepth=6)
    B, T, D = x.shape
    K = w.shape[0]
    plan = Plan(K, levels, mat, lead, slack, Q, opts.get("tail_len", 36), opts.get("unst", 3), opts.get("cap_add", 0),
                opts.get("xstage", True), opts.get("xunst", True), opts.get("head", True), opts.get("raw_ok", True))
    P = plan.P
    TM = 2 * P * Q
    nt = pl.cdiv(T, TM)
    assert TM % HALO == 0
    hb = TM // HALO
    QS = Q + 4
    ng = len(plan.g_terms)
    NS = opts.get("ns", 8)
    opts = dict(opts, ns=NS, nblk=nt, nb=B)
    N = B * nt

    assert not plan.xstage and plan.xunst and nt >= 3 and T % 16 == 0 and T - (nt - 1) * TM >= HALO
    return pl.pallas_call(
        functools.partial(_kernel, plan=plan, Q=Q, K=K, D=D, T=T, opts=opts),
        in_specs=[pl.BlockSpec(memory_space=pl.ANY), pl.BlockSpec(memory_space=pl.ANY)],
        out_specs=pl.BlockSpec(memory_space=pl.ANY),
        out_shape=jax.ShapeDtypeStruct((B, T, D), x.dtype),
        scratch_shapes=[
            pltpu.VMEM((2, P * QS + 8, 128), jnp.uint32),
            pltpu.VMEM((ng, 2 * D // 128, D // 2, 128), jnp.uint32),
            pltpu.VMEM((max(plan.n_in, 1), 2, 2, Q, 128), jnp.float32),
            pltpu.VMEM((max(plan.n_out, 1), 2 * Q, 2 * D), jnp.float32),
            pltpu.VMEM((2, P * QS, 128), jnp.uint32),
            pltpu.VMEM((K, D, 2 * D), w.dtype),
            pltpu.VMEM((2, HALO + TM, D), x.dtype),
            pltpu.VMEM((2, TM, D), x.dtype),
            pltpu.SemaphoreType.DMA((NS,)),
            pltpu.SemaphoreType.DMA((2, 2)),
            pltpu.SemaphoreType.DMA((2,)),
        ],
        compiler_params=pltpu.CompilerParams(
            vmem_limit_bytes=124 * 1024 * 1024),
    )(x, w)
```

```python
import functools
import math

import jax
import jax.numpy as jnp
import jax.experimental.pallas as pl
import jax.experimental.pallas.tpu as pltpu

_LEVELS = "WBBKK"
_MATERIALISE = (1, 2, 3)
_Q = 24
_HALO = 64
_HALO32 = _HALO // 2
_W_SLABS = 16
_W_DEPTH = 6
_LANES = 128


class _Node:
    def __init__(self, kind, parent, taps, nout, path):
        self.kind, self.parent, self.taps, self.nout, self.path = kind, parent, taps, nout, path
        self.depth = len(path)
        self.children = None

    def din(self, r):
        h = self.nout
        return {
            "K0": [(1, 2 * r), (-1, 2 * r + 1)], "Km": [(1, 2 * r + 1)], "K1": [(1, 2 * r + 2), (-1, 2 * r + 1)],
            "B0": [(1, r), (-1, h + r)], "Bm": [(1, h + r)], "B1": [(1, 2 * h + r), (-1, h + r)],
            "W0": [(1, r), (-1, 2 * h + r)], "W1": [(1, h + r), (1, 2 * h + r)],
            "W2": [(1, 2 * h + r), (-1, h + r)], "W3": [(1, 3 * h + r), (-1, h + r)],
        }[self.kind]


def _tap_sum(a, b, sign=1):
    return {**a, **{k: sign * v for k, v in b.items()}}


def _build_tree(ktaps, levels):
    nout = math.prod(3 if lv == "W" else 2 for lv in levels)
    root = _Node("root", None, [{k: 1} for k in range(ktaps)], nout, ())

    def split(n, rest):
        if not rest:
            return
        lv = rest[0]
        if lv == "K":
            h, lo, hi = n.nout // 2, n.taps[0::2], n.taps[1::2]
        else:
            h = n.nout // (3 if lv == "W" else 2)
            lo, hi = n.taps[:h], n.taps[h:]
        mix = lambda sign: [_tap_sum(a, hi[j], sign) if j < len(hi) else a for j, a in enumerate(lo)]
        if lv == "W":
            kids = [("W0", lo), ("W1", mix(1)), ("W2", mix(-1)), ("W3", hi)]
        else:
            kids = [(lv + "0", lo), (lv + "m", mix(1)), (lv + "1", hi)]
        n.children = [_Node(k, n, t, h, n.path + (i,)) for i, (k, t) in enumerate(kids)]
        for c in n.children:
            split(c, rest[1:])

    split(root, levels)
    return root


class _Plan:
    def __init__(self, ktaps, levels, materialise, q):
        self.root = _build_tree(ktaps, levels)
        self.P = self.root.nout
        self.materialise = materialise
        self.items = []
        self._arrays = 0
        self._output_network()
        self._input_network(q)

    def _new(self, n):
        self._arrays += n
        return list(range(self._arrays - n, self._arrays))

    def _solve(self, n, inits, sinks):
        if n.children is None:
            self.items.append(("leaf", n, inits[0], sinks[0]))
            return
        c0, cm, c1 = n.children
        half = n.nout // 2
        mids = self._new(half)
        self._solve(cm, [[] for _ in mids], [("store", m) for m in mids])
        i0, i1 = (range(half), range(half, n.nout)) if c0.kind == "B0" else (range(0, n.nout, 2), range(1, n.nout, 2))
        for c, idx in ((c0, i0), (c1, i1)):
            self._solve(c, [inits[i] + [m] for i, m in zip(idx, mids)], [sinks[i] for i in idx])

    def _output_network(self):
        w0, w1, w2, w3 = self.root.children
        h = self.P // 3
        m1, s = self._new(h), self._new(h)
        self._solve(w1, [[] for _ in m1], [("store", m) for m in m1])
        self._solve(w2, [[m] for m in m1], [("half", a) for a in s])
        head, n0 = self.items, len(self.items)
        self._solve(w0, [[a] for a in s], [("final", i) for i in range(h)])
        self._solve(w3, [[a] for a in s], [("final", 2 * h + i) for i in range(h)])
        combs = [("comb", None, (m1[i], s[i]), ("final", h + i)) for i in range(h)]
        rest = head[n0:]
        self.items = head[:n0]
        every = max(1, len(rest) // (h + 1))
        for i, it in enumerate(rest):
            self.items.append(it)
            if (i + 1) % every == 0 and combs:
                self.items.append(combs.pop(0))
        self.items += combs

    def _expr(self, n, r):
        return [(s * s2, src) for s, pr in n.din(r) for s2, src in self._resolve(n.parent, pr)]

    def _resolve(self, n, r):
        if n.parent is None:
            return [(1, ("x", r))]
        e = self._expr(n, r)
        if n.depth not in self.materialise or (len(e) == 1 and e[0][0] == 1):
            return e
        key = ("a", n.path, r)
        self.prep_expr[key] = e
        return [(1, key)]

    def _input_network(self, q):
        items, n = self.items, len(self.items)
        self.prep_expr, self.leaf_expr, deadline = {}, {}, {}
        for i, it in enumerate(items):
            if it[0] == "leaf" and it[1].taps:
                self.leaf_expr[it[1].path] = e = self._expr(it[1], 0)
                for _, src in e:
                    deadline.setdefault(src, i)
        cap = max(1, math.ceil(1.15 * len(self.prep_expr) / n))
        load, slot = {}, {}
        depth = lambda key: len(key[1])
        for d in sorted(set(map(depth, self.prep_expr)), reverse=True):
            for k in sorted((k for k in self.prep_expr if depth(k) == d), key=lambda k: -deadline[k]):
                s = max(deadline[k] - 1, 0)
                while s > 0 and load.get(s, 0) >= cap:
                    s -= 1
                slot[k] = s
                load[s] = load.get(s, 0) + 1
                for _, src in self.prep_expr[k]:
                    if src[0] == "a":
                        deadline[src] = min(deadline.get(src, n), s)
        before = [[] for _ in range(n)]
        for k in sorted(slot, key=lambda k: (slot[k], depth(k))):
            before[slot[k]].append(("prep", k))
        first_final = min(i for i, it in enumerate(items) if it[3][0] == "final")
        unstage = [("unstage", c, i) for i in range(q) for c in range(2)]
        for i, op in enumerate(unstage):
            before[3 + i * (first_final - 11) // len(unstage)].append(op)
        self.unstage = unstage
        self.ops = [("halo", c, 0) for c in range(2)] + [("stage", c, i) for i in range(q) for c in range(2)]
        body = [op for b, it in zip(before, items) for op in b + [it]]
        self.ops += body

        last_in, last_out = {}, {}
        for t, op in enumerate(body):
            if op[0] == "prep":
                last_in.update({src: t for _, src in self.prep_expr[op[1]] if src[0] == "a"})
            elif op[0] == "leaf":
                last_in.update({src: t for _, src in self.leaf_expr.get(op[1].path, ())})
            if op[0] in ("leaf", "comb"):
                last_out.update({a: t for a in op[2]})

        def allocate(defs, last):
            slots, free, pending, count, release = {}, [], [], 0, {}
            for k, t in last.items():
                release.setdefault(t, []).append(k)
            for t, k in enumerate(defs):
                if k is not None:
                    if not free:
                        free.append(count)
                        count += 1
                    slots[k] = free.pop(0)
                pending += [(t, r) for r in release.get(t, [])]
                while pending and pending[0][0] <= t - 2:
                    free.append(slots[pending.pop(0)[1]])
            return slots, max(count, 1)

        self.in_slot, self.n_in = allocate([op[1] if op[0] == "prep" else None for op in body], last_in)
        self.out_slot, self.n_out = allocate(
            [op[3][1] if op[0] in ("leaf", "comb") and op[3][0] != "final" else None for op in body], last_out)

        self.g_slot, self.g_raw = {}, {}
        for it in items:
            if it[0] == "leaf" and it[1].taps:
                (tap,) = it[1].taps
                if it[1].path[0] in (0, 3) and len(tap) == 1:
                    (self.g_raw[it[1].path],) = tap
                else:
                    self.g_slot[it[1].path] = len(self.g_slot)


def _pack(lo, hi):
    return pltpu.pack_elementwise([lo, hi], packed_dtype=jnp.bfloat16)


def _unpack(v):
    return pltpu.bitcast(v << 16, jnp.float32), pltpu.bitcast(v & jnp.uint32(0xFFFF0000), jnp.float32)


def _signed_sum(terms):
    pos = [v for s, v in terms if s > 0]
    neg = [v for s, v in terms if s < 0]
    parts = []
    while pos and neg:
        parts.append(pos.pop(0) - neg.pop(0))
    parts += pos
    while len(parts) > 1:
        parts = [parts[i] + parts[i + 1] if i + 1 < len(parts) else parts[i] for i in range(0, len(parts), 2)]
    acc = parts[0]
    for v in neg:
        acc = acc - v
    return acc


def _kernel(x_hbm, w_hbm, o_hbm, pm_ref, g_ref, a_ref, b_ref, po_ref, w_ref, x_buf, o_buf, w_sem, x_sem, o_sem,
            *, plan, nb, T, K, D, nblk):
    P, Q = plan.P, _Q
    QS = Q + 4
    TM = 2 * P * Q
    N = nb * nblk
    RW = D // _W_SLABS
    halves, ntiles = D // _LANES, 2 * D // _LANES
    lanes = lambda c: slice(c * _LANES, (c + 1) * _LANES)
    zero = jnp.int32(0)

    def row0(t):
        return pl.multiple_of(jnp.where(t > 0, T - (nblk - t) * TM, 0), 16)

    def x_copies(b, t, slot):
        t0 = row0(t)
        h0 = pl.multiple_of(jnp.maximum(t0 - _HALO, 0), 16)
        return (pltpu.make_async_copy(x_hbm.at[b, pl.ds(h0, _HALO), :], x_buf.at[slot, pl.ds(0, _HALO), :],
                                      x_sem.at[slot, 0]),
                pltpu.make_async_copy(x_hbm.at[b, pl.ds(t0, TM), :], x_buf.at[slot, pl.ds(_HALO, TM), :],
                                      x_sem.at[slot, 1]))

    def o_copy(b, t, slot):
        return pltpu.make_async_copy(o_buf.at[slot], o_hbm.at[b, pl.ds(row0(t), TM), :], o_sem.at[slot])

    def w_copy(i):
        r = pl.ds(pl.multiple_of(i * RW, RW), RW)
        return pltpu.make_async_copy(w_hbm.at[:, r, :], w_ref.at[:, r, :], w_sem.at[i])

    def g_tap(n, load_tap, memo, j):
        key = (n.path, j)
        if key not in memo:
            f32 = lambda v: _unpack(v[1]) if v[0] == "w" else v[1:]
            k, par = n.kind, n.parent
            if k == "root":
                out = ("w", load_tap(j))
            elif k in ("K0", "K1", "B0", "B1", "W0", "W3"):
                jp = {"K0": 2 * j, "K1": 2 * j + 1, "B0": j, "W0": j, "B1": n.nout + j, "W3": n.nout + j}[k]
                out = g_tap(par, load_tap, memo, jp)
            else:
                j0, j1 = (2 * j, 2 * j + 1) if k == "Km" else (j, n.nout + j)
                out = g_tap(par, load_tap, memo, j0)
                if j1 < len(par.taps):
                    (l0, h0), (l1, h1) = f32(out), f32(g_tap(par, load_tap, memo, j1))
                    out = ("f", l0 - l1, h0 - h1) if k == "W2" else ("f", l0 + l1, h0 + h1)
                elif k[0] == "W":
                    out = ("f",) + tuple(f32(out))
            memo[key] = out
        return memo[key]

    def g_leaves(n):
        if n.children is None:
            return [n] if n.path in plan.g_slot else []
        order = (1, 2, 0, 3) if n.parent is None else (0, 2, 1)
        return [lf for i in order for lf in g_leaves(n.children[i])]

    def transform_slab(i, copy_next):
        w_copy(i).wait()
        if copy_next:
            w_copy(i + _W_DEPTH).start()
        r0 = pl.multiple_of(i * RW, 16)
        s0 = pl.multiple_of(i * (RW // 2), 8)
        for nt in range(ntiles):
            memo, top = {}, None
            for lf in g_leaves(plan.root):
                if lf.path[:2] != top:
                    top, memo = lf.path[:2], {}
                load_tap = lambda k: pltpu.bitcast(w_ref[k, pl.ds(r0, 16), lanes(nt)], jnp.uint32)
                v = g_tap(lf, load_tap, memo, 0)
                g_ref[plan.g_slot[lf.path], nt, pl.ds(s0, 8), :] = v[1] if v[0] == "w" else _pack(v[1], v[2])
        return 0

    off0 = _HALO32 - (K - 1) + (P - _HALO32)

    def load(src, c):
        if src[0] == "x":
            rho = src[1] + off0
            return _unpack(pm_ref[c, pl.ds((rho % P) * QS + rho // P, Q), :])
        sl = plan.in_slot[src]
        return a_ref[sl, c, 0], a_ref[sl, c, 1]

    def evaluate(e, c):
        vals = [(s, load(src, c)) for s, src in e]
        return _signed_sum([(s, v[0]) for s, v in vals]), _signed_sum([(s, v[1]) for s, v in vals])

    def sink(y, to):
        if to[0] == "final":
            tf = jnp.tanh(y[:, :D])
            o = (0.5 * (tf * jnp.tanh(0.5 * y[:, D:]) + tf)).astype(jnp.bfloat16)
            for c in range(halves):
                po_ref[c, pl.ds(to[1] * QS, Q), :] = pltpu.bitcast(o[:, lanes(c)], jnp.uint32)
        else:
            b_ref[plan.out_slot[to[1]]] = y if to[0] == "store" else 0.5 * y

    def emit(ops, keep_halo, slot):
        for op in ops:
            kind = op[0]
            if kind == "prep":
                sl = plan.in_slot[op[1]]
                for c in range(halves):
                    a_ref[sl, c, 0], a_ref[sl, c, 1] = evaluate(plan.prep_expr[op[1]], c)
            elif kind == "leaf":
                _, n, inits, to = op
                acc = None
                for a in inits:
                    v = b_ref[plan.out_slot[a]]
                    acc = v if acc is None else acc + v
                if n.taps:
                    lhs = jnp.concatenate(
                        [pltpu.bitcast(_pack(*evaluate(plan.leaf_expr[n.path], c)), jnp.bfloat16)
                         for c in range(halves)], axis=1)
                    if n.path in plan.g_raw:
                        rhs = w_ref[plan.g_raw[n.path]]
                    else:
                        rhs = jnp.concatenate([pltpu.bitcast(g_ref[plan.g_slot[n.path], nt], jnp.bfloat16)
                                               for nt in range(ntiles)], axis=1)
                    prod = jnp.dot(lhs, rhs, preferred_element_type=jnp.float32)
                    acc = prod if acc is None else acc + prod
                sink(acc, to)
            elif kind == "comb":
                _, _, (m1, s), to = op
                sink(b_ref[plan.out_slot[m1]] - b_ref[plan.out_slot[s]], to)
            elif kind == "halo":
                c = op[1]
                halo = pltpu.bitcast(x_buf[slot, pl.ds(0, _HALO), lanes(c)], jnp.uint32)
                pm_ref[c, pl.ds((P - _HALO32) * QS, _HALO32, stride=QS), :] = jnp.where(
                    keep_halo, halo, jnp.zeros_like(halo))
            elif kind == "stage":
                _, c, i = op
                pm_ref[c, pl.ds(i + 1, P, stride=QS), :] = pltpu.bitcast(
                    x_buf[slot, pl.ds(_HALO + 2 * P * i, 2 * P), lanes(c)], jnp.uint32)
            else:
                _, c, i = op
                o_buf[slot, pl.ds(2 * P * i, 2 * P), lanes(c)] = pltpu.bitcast(
                    po_ref[c, pl.ds(i, P, stride=QS), :], jnp.bfloat16)

    for i in range(_W_DEPTH):
        w_copy(i).start()
    po_ref[...] = jnp.zeros(po_ref.shape, po_ref.dtype)
    o_buf[1] = jnp.zeros(o_buf.shape[1:], o_buf.dtype)
    jax.lax.fori_loop(0, _W_SLABS - _W_DEPTH, lambda i, _: transform_slab(i, True), 0)
    for cp in x_copies(zero, zero, 0):
        cp.start()
    o_copy(zero, zero, 1).start()
    jax.lax.fori_loop(_W_SLABS - _W_DEPTH, _W_SLABS, lambda i, _: transform_slab(i, False), 0)

    def block(n, carry):
        b, t, pb, pt = carry
        slot = n & 1
        wrap, last = t == nblk - 1, n == N - 1
        nxt_b = jnp.where(last, b, jnp.where(wrap, b + 1, b))
        nxt_t = jnp.where(last, t, jnp.where(wrap, 0, t + 1))
        for cp in x_copies(b, t, slot):
            cp.wait()
        for cp in x_copies(nxt_b, nxt_t, 1 - slot):
            cp.start()
        emit(plan.ops, t > 0, slot)
        o_copy(pb, pt, 1 - slot).wait()
        o_copy(pb, pt, slot).start()
        return nxt_b, nxt_t, b, t

    b, t, pb, pt = jax.lax.fori_loop(0, N, block, (zero, zero, zero, zero))
    slot = N & 1
    emit(plan.unstage, False, slot)
    o_copy(pb, pt, slot).start()
    for cp in x_copies(b, t, slot):
        cp.wait()
    o_copy(pb, pt, 1 - slot).wait()
    o_copy(pb, pt, slot).wait()


@jax.jit
def pallas_standalone__autoregressive_conv_wavernn__speech_kernel(x: jax.Array, w: jax.Array):
    B, T, D = x.shape
    K = w.shape[0]
    plan = _Plan(K, _LEVELS, _MATERIALISE, _Q)
    P, Q = plan.P, _Q
    TM = 2 * P * Q
    nblk = pl.cdiv(T, TM)
    assert D == 2 * _LANES and K - 1 <= _HALO32 <= P and D % (16 * _W_SLABS) == 0
    assert nblk >= 3 and T % 16 == 0 and T - (nblk - 1) * TM >= _HALO
    return pl.pallas_call(
        functools.partial(_kernel, plan=plan, nb=B, T=T, K=K, D=D, nblk=nblk),
        in_specs=[pl.BlockSpec(memory_space=pl.ANY), pl.BlockSpec(memory_space=pl.ANY)],
        out_specs=pl.BlockSpec(memory_space=pl.ANY),
        out_shape=jax.ShapeDtypeStruct((B, T, D), x.dtype),
        scratch_shapes=[
            pltpu.VMEM((2, P * (Q + 4) + 8, _LANES), jnp.uint32),
            pltpu.VMEM((len(plan.g_slot), 2 * D // _LANES, D // 2, _LANES), jnp.uint32),
            pltpu.VMEM((plan.n_in, 2, 2, Q, _LANES), jnp.float32),
            pltpu.VMEM((plan.n_out, 2 * Q, 2 * D), jnp.float32),
            pltpu.VMEM((2, P * (Q + 4), _LANES), jnp.uint32),
            pltpu.VMEM((K, D, 2 * D), w.dtype),
            pltpu.VMEM((2, _HALO + TM, D), x.dtype),
            pltpu.VMEM((2, TM, D), x.dtype),
            pltpu.SemaphoreType.DMA((_W_SLABS,)),
            pltpu.SemaphoreType.DMA((2, 2)),
            pltpu.SemaphoreType.DMA((2,)),
        ],
        compiler_params=pltpu.CompilerParams(vmem_limit_bytes=124 * 1024 * 1024),
    )(x, w)
```

```python
import functools
import math

import jax
import jax.numpy as jnp
import jax.experimental.pallas as pl
import jax.experimental.pallas.tpu as pltpu

_LEVELS = "WBBKK"
_MATERIALISE = (1, 2, 3)
_Q = 24
_HALO = 64
_HALO32 = _HALO // 2
_W_SLABS = 16
_W_DEPTH = 6
_LANES = 128


class _Node:
    def __init__(self, kind, parent, taps, nout, path):
        self.kind, self.parent, self.taps, self.nout, self.path = kind, parent, taps, nout, path
        self.depth = len(path)
        self.children = None

    def din(self, r):
        h = self.nout
        return {
            "K0": [(1, 2 * r), (-1, 2 * r + 1)], "Km": [(1, 2 * r + 1)], "K1": [(1, 2 * r + 2), (-1, 2 * r + 1)],
            "B0": [(1, r), (-1, h + r)], "Bm": [(1, h + r)], "B1": [(1, 2 * h + r), (-1, h + r)],
            "W0": [(1, r), (-1, 2 * h + r)], "W1": [(1, h + r), (1, 2 * h + r)],
            "W2": [(1, 2 * h + r), (-1, h + r)], "W3": [(1, 3 * h + r), (-1, h + r)],
        }[self.kind]


def _tap_sum(a, b, sign=1):
    return {**a, **{k: sign * v for k, v in b.items()}}


def _build_tree(ktaps, levels):
    nout = math.prod(3 if lv == "W" else 2 for lv in levels)
    root = _Node("root", None, [{k: 1} for k in range(ktaps)], nout, ())

    def split(n, rest):
        if not rest:
            return
        lv = rest[0]
        if lv == "K":
            h, lo, hi = n.nout // 2, n.taps[0::2], n.taps[1::2]
        else:
            h = n.nout // (3 if lv == "W" else 2)
            lo, hi = n.taps[:h], n.taps[h:]
        mix = lambda sign: [_tap_sum(a, hi[j], sign) if j < len(hi) else a for j, a in enumerate(lo)]
        if lv == "W":
            kids = [("W0", lo), ("W1", mix(1)), ("W2", mix(-1)), ("W3", hi)]
        else:
            kids = [(lv + "0", lo), (lv + "m", mix(1)), (lv + "1", hi)]
        n.children = [_Node(k, n, t, h, n.path + (i,)) for i, (k, t) in enumerate(kids)]
        for c in n.children:
            split(c, rest[1:])

    split(root, levels)
    return root


class _Plan:
    def __init__(self, ktaps, levels, materialise, q):
        self.root = _build_tree(ktaps, levels)
        self.P = self.root.nout
        self.materialise = materialise
        self.items = []
        self._arrays = 0
        self._output_network()
        self._input_network(q)

    def _new(self, n):
        self._arrays += n
        return list(range(self._arrays - n, self._arrays))

    def _solve(self, n, inits, sinks):
        if n.children is None:
            self.items.append(("leaf", n, inits[0], sinks[0]))
            return
        c0, cm, c1 = n.children
        half = n.nout // 2
        mids = self._new(half)
        self._solve(cm, [[] for _ in mids], [("store", m) for m in mids])
        i0, i1 = (range(half), range(half, n.nout)) if c0.kind == "B0" else (range(0, n.nout, 2), range(1, n.nout, 2))
        for c, idx in ((c0, i0), (c1, i1)):
            self._solve(c, [inits[i] + [m] for i, m in zip(idx, mids)], [sinks[i] for i in idx])

    def _output_network(self):
        w0, w1, w2, w3 = self.root.children
        h = self.P // 3
        m1, s = self._new(h), self._new(h)
        self._solve(w1, [[] for _ in m1], [("store", m) for m in m1])
        self._solve(w2, [[m] for m in m1], [("half", a) for a in s])
        head, n0 = self.items, len(self.items)
        self._solve(w0, [[a] for a in s], [("final", i) for i in range(h)])
        self._solve(w3, [[a] for a in s], [("final", 2 * h + i) for i in range(h)])
        combs = [("comb", None, (m1[i], s[i]), ("final", h + i)) for i in range(h)]
        rest = head[n0:]
        self.items = head[:n0]
        every = max(1, len(rest) // (h + 1))
        for i, it in enumerate(rest):
            self.items.append(it)
            if (i + 1) % every == 0 and combs:
                self.items.append(combs.pop(0))
        self.items += combs

    def _expr(self, n, r):
        return [(s * s2, src) for s, pr in n.din(r) for s2, src in self._resolve(n.parent, pr)]

    def _resolve(self, n, r):
        if n.parent is None:
            return [(1, ("x", r))]
        e = self._expr(n, r)
        if n.depth not in self.materialise or (len(e) == 1 and e[0][0] == 1):
            return e
        key = ("a", n.path, r)
        self.prep_expr[key] = e
        return [(1, key)]

    def _input_network(self, q):
        items, n = self.items, len(self.items)
        self.prep_expr, self.leaf_expr, deadline = {}, {}, {}
        for i, it in enumerate(items):
            if it[0] == "leaf" and it[1].taps:
                self.leaf_expr[it[1].path] = e = self._expr(it[1], 0)
                for _, src in e:
                    deadline.setdefault(src, i)
        cap = max(1, math.ceil(1.15 * len(self.prep_expr) / n))
        load, slot = {}, {}
        depth = lambda key: len(key[1])
        for d in sorted(set(map(depth, self.prep_expr)), reverse=True):
            for k in sorted((k for k in self.prep_expr if depth(k) == d), key=lambda k: -deadline[k]):
                s = max(deadline[k] - 1, 0)
                while s > 0 and load.get(s, 0) >= cap:
                    s -= 1
                slot[k] = s
                load[s] = load.get(s, 0) + 1
                for _, src in self.prep_expr[k]:
                    if src[0] == "a":
                        deadline[src] = min(deadline.get(src, n), s)
        before = [[] for _ in range(n)]
        for k in sorted(slot, key=lambda k: (slot[k], depth(k))):
            before[slot[k]].append(("prep", k))
        first_final = min(i for i, it in enumerate(items) if it[3][0] == "final")
        unstage = [("unstage", c, i) for i in range(q) for c in range(2)]
        for i, op in enumerate(unstage):
            before[3 + i * (first_final - 11) // len(unstage)].append(op)
        self.unstage = unstage
        self.ops = [("halo", c, 0) for c in range(2)] + [("stage", c, i) for i in range(q) for c in range(2)]
        body = [op for b, it in zip(before, items) for op in b + [it]]
        self.ops += body

        last_in, last_out = {}, {}
        for t, op in enumerate(body):
            if op[0] == "prep":
                last_in.update({src: t for _, src in self.prep_expr[op[1]] if src[0] == "a"})
            elif op[0] == "leaf":
                last_in.update({src: t for _, src in self.leaf_expr.get(op[1].path, ())})
            if op[0] in ("leaf", "comb"):
                last_out.update({a: t for a in op[2]})

        def allocate(defs, last):
            slots, free, pending, count, release = {}, [], [], 0, {}
            for k, t in last.items():
                release.setdefault(t, []).append(k)
            for t, k in enumerate(defs):
                if k is not None:
                    if not free:
                        free.append(count)
                        count += 1
                    slots[k] = free.pop(0)
                pending += [(t, r) for r in release.get(t, [])]
                while pending and pending[0][0] <= t - 2:
                    free.append(slots[pending.pop(0)[1]])
            return slots, max(count, 1)

        self.in_slot, self.n_in = allocate([op[1] if op[0] == "prep" else None for op in body], last_in)
        self.out_slot, self.n_out = allocate(
            [op[3][1] if op[0] in ("leaf", "comb") and op[3][0] != "final" else None for op in body], last_out)

        self.g_slot, self.g_raw = {}, {}
        for it in items:
            if it[0] == "leaf" and it[1].taps:
                (tap,) = it[1].taps
                if it[1].path[0] in (0, 3) and len(tap) == 1:
                    (self.g_raw[it[1].path],) = tap
                else:
                    self.g_slot[it[1].path] = len(self.g_slot)


def _pack(lo, hi):
    return pltpu.pack_elementwise([lo, hi], packed_dtype=jnp.bfloat16)


def _unpack(v):
    return pltpu.bitcast(v << 16, jnp.float32), pltpu.bitcast(v & jnp.uint32(0xFFFF0000), jnp.float32)


def _signed_sum(terms):
    pos = [v for s, v in terms if s > 0]
    neg = [v for s, v in terms if s < 0]
    parts = []
    while pos and neg:
        parts.append(pos.pop(0) - neg.pop(0))
    parts += pos
    while len(parts) > 1:
        parts = [parts[i] + parts[i + 1] if i + 1 < len(parts) else parts[i] for i in range(0, len(parts), 2)]
    acc = parts[0]
    for v in neg:
        acc = acc - v
    return acc


def _kernel(x_hbm, w_hbm, o_hbm, pm_ref, g_ref, a_ref, b_ref, po_ref, w_ref, x_buf, o_buf, w_sem, x_sem, o_sem,
            *, plan, nb, T, K, D, nblk):
    P, Q = plan.P, _Q
    QS = Q + 4
    TM = 2 * P * Q
    N = nb * nblk
    RW = D // _W_SLABS
    halves, ntiles = D // _LANES, 2 * D // _LANES
    lanes = lambda c: slice(c * _LANES, (c + 1) * _LANES)
    zero = jnp.int32(0)

    def row0(t):
        return pl.multiple_of(jnp.where(t > 0, T - (nblk - t) * TM, 0), 16)

    def x_copies(b, t, slot):
        t0 = row0(t)
        h0 = pl.multiple_of(jnp.maximum(t0 - _HALO, 0), 16)
        return (pltpu.make_async_copy(x_hbm.at[b, pl.ds(h0, _HALO), :], x_buf.at[slot, pl.ds(0, _HALO), :],
                                      x_sem.at[slot, 0]),
                pltpu.make_async_copy(x_hbm.at[b, pl.ds(t0, TM), :], x_buf.at[slot, pl.ds(_HALO, TM), :],
                                      x_sem.at[slot, 1]))

    def o_copy(b, t, slot):
        return pltpu.make_async_copy(o_buf.at[slot], o_hbm.at[b, pl.ds(row0(t), TM), :], o_sem.at[slot])

    def w_copy(i):
        r = pl.ds(pl.multiple_of(i * RW, RW), RW)
        return pltpu.make_async_copy(w_hbm.at[:, r, :], w_ref.at[:, r, :], w_sem.at[i])

    def g_tap(n, load_tap, memo, j):
        key = (n.path, j)
        if key not in memo:
            f32 = lambda v: _unpack(v[1]) if v[0] == "w" else v[1:]
            k, par = n.kind, n.parent
            if k == "root":
                out = ("w", load_tap(j))
            elif k in ("K0", "K1", "B0", "B1", "W0", "W3"):
                jp = {"K0": 2 * j, "K1": 2 * j + 1, "B0": j, "W0": j, "B1": n.nout + j, "W3": n.nout + j}[k]
                out = g_tap(par, load_tap, memo, jp)
            else:
                j0, j1 = (2 * j, 2 * j + 1) if k == "Km" else (j, n.nout + j)
                out = g_tap(par, load_tap, memo, j0)
                if j1 < len(par.taps):
                    (l0, h0), (l1, h1) = f32(out), f32(g_tap(par, load_tap, memo, j1))
                    out = ("f", l0 - l1, h0 - h1) if k == "W2" else ("f", l0 + l1, h0 + h1)
                elif k[0] == "W":
                    out = ("f",) + tuple(f32(out))
            memo[key] = out
        return memo[key]

    def g_leaves(n):
        if n.children is None:
            return [n] if n.path in plan.g_slot else []
        order = (1, 2, 0, 3) if n.parent is None else (2, 0, 1)
        return [lf for i in order for lf in g_leaves(n.children[i])]

    def transform_slab(i, copy_next):
        w_copy(i).wait()
        if copy_next:
            w_copy(i + _W_DEPTH).start()
        r0 = pl.multiple_of(i * RW, 16)
        s0 = pl.multiple_of(i * (RW // 2), 8)
        for nt in range(ntiles):
            memo, top = {}, None
            for lf in g_leaves(plan.root):
                if lf.path[:2] != top:
                    top, memo = lf.path[:2], {}
                load_tap = lambda k: pltpu.bitcast(w_ref[k, pl.ds(r0, 16), lanes(nt)], jnp.uint32)
                v = g_tap(lf, load_tap, memo, 0)
                g_ref[plan.g_slot[lf.path], nt, pl.ds(s0, 8), :] = v[1] if v[0] == "w" else _pack(v[1], v[2])
        return 0

    off0 = _HALO32 - (K - 1) + (P - _HALO32)

    def load(src, c):
        if src[0] == "x":
            rho = src[1] + off0
            return _unpack(pm_ref[c, pl.ds((rho % P) * QS + rho // P, Q), :])
        sl = plan.in_slot[src]
        return a_ref[sl, c, 0], a_ref[sl, c, 1]

    def evaluate(e, c):
        vals = [(s, load(src, c)) for s, src in e]
        return _signed_sum([(s, v[0]) for s, v in vals]), _signed_sum([(s, v[1]) for s, v in vals])

    def sink(y, to):
        if to[0] == "final":
            tf = jnp.tanh(y[:, :D])
            o = (0.5 * (tf * jnp.tanh(0.5 * y[:, D:]) + tf)).astype(jnp.bfloat16)
            for c in range(halves):
                po_ref[c, pl.ds(to[1] * QS, Q), :] = pltpu.bitcast(o[:, lanes(c)], jnp.uint32)
        else:
            b_ref[plan.out_slot[to[1]]] = y if to[0] == "store" else 0.5 * y

    def emit(ops, keep_halo, slot):
        for op in ops:
            kind = op[0]
            if kind == "prep":
                sl = plan.in_slot[op[1]]
                for c in range(halves):
                    a_ref[sl, c, 0], a_ref[sl, c, 1] = evaluate(plan.prep_expr[op[1]], c)
            elif kind == "leaf":
                _, n, inits, to = op
                acc = None
                for a in inits:
                    v = b_ref[plan.out_slot[a]]
                    acc = v if acc is None else acc + v
                if n.taps:
                    lhs = jnp.concatenate(
                        [pltpu.bitcast(_pack(*evaluate(plan.leaf_expr[n.path], c)), jnp.bfloat16)
                         for c in range(halves)], axis=1)
                    if n.path in plan.g_raw:
                        rhs = w_ref[plan.g_raw[n.path]]
                    else:
                        rhs = jnp.concatenate([pltpu.bitcast(g_ref[plan.g_slot[n.path], nt], jnp.bfloat16)
                                               for nt in range(ntiles)], axis=1)
                    prod = jnp.dot(lhs, rhs, preferred_element_type=jnp.float32)
                    acc = prod if acc is None else acc + prod
                sink(acc, to)
            elif kind == "comb":
                _, _, (m1, s), to = op
                sink(b_ref[plan.out_slot[m1]] - b_ref[plan.out_slot[s]], to)
            elif kind == "halo":
                c = op[1]
                halo = pltpu.bitcast(x_buf[slot, pl.ds(0, _HALO), lanes(c)], jnp.uint32)
                pm_ref[c, pl.ds((P - _HALO32) * QS, _HALO32, stride=QS), :] = jnp.where(
                    keep_halo, halo, jnp.zeros_like(halo))
            elif kind == "stage":
                _, c, i = op
                pm_ref[c, pl.ds(i + 1, P, stride=QS), :] = pltpu.bitcast(
                    x_buf[slot, pl.ds(_HALO + 2 * P * i, 2 * P), lanes(c)], jnp.uint32)
            else:
                _, c, i = op
                o_buf[slot, pl.ds(2 * P * i, 2 * P), lanes(c)] = pltpu.bitcast(
                    po_ref[c, pl.ds(i, P, stride=QS), :], jnp.bfloat16)

    for i in range(_W_DEPTH):
        w_copy(i).start()
    po_ref[...] = jnp.zeros(po_ref.shape, po_ref.dtype)
    jax.lax.fori_loop(0, _W_SLABS - _W_DEPTH, lambda i, _: transform_slab(i, True), 0)
    for cp in x_copies(zero, zero, 0):
        cp.start()
    jax.lax.fori_loop(_W_SLABS - _W_DEPTH, _W_SLABS, lambda i, _: transform_slab(i, False), 0)

    def block(n, carry):
        b, t, pb, pt = carry
        slot = n & 1
        wrap, last = t == nblk - 1, n == N - 1
        nxt_b = jnp.where(last, b, jnp.where(wrap, b + 1, b))
        nxt_t = jnp.where(last, t, jnp.where(wrap, 0, t + 1))
        for cp in x_copies(b, t, slot):
            cp.wait()
        for cp in x_copies(nxt_b, nxt_t, 1 - slot):
            cp.start()
        emit(plan.ops, t > 0, slot)
        pl.when(n >= 2)(lambda: o_copy(pb, pt, 1 - slot).wait())
        pl.when(n >= 1)(lambda: o_copy(pb, pt, slot).start())
        return nxt_b, nxt_t, b, t

    b, t, pb, pt = jax.lax.fori_loop(0, N, block, (zero, zero, zero, zero))
    slot = N & 1
    emit(plan.unstage, False, slot)
    o_copy(pb, pt, slot).start()
    for cp in x_copies(b, t, slot):
        cp.wait()
    o_copy(pb, pt, 1 - slot).wait()
    o_copy(pb, pt, slot).wait()


@jax.jit
def pallas_standalone__autoregressive_conv_wavernn__speech_kernel(x: jax.Array, w: jax.Array):
    B, T, D = x.shape
    K = w.shape[0]
    plan = _Plan(K, _LEVELS, _MATERIALISE, _Q)
    P, Q = plan.P, _Q
    TM = 2 * P * Q
    nblk = pl.cdiv(T, TM)
    assert D == 2 * _LANES and K - 1 <= _HALO32 <= P and D % (16 * _W_SLABS) == 0
    assert nblk >= 3 and T % 16 == 0 and T - (nblk - 1) * TM >= _HALO
    return pl.pallas_call(
        functools.partial(_kernel, plan=plan, nb=B, T=T, K=K, D=D, nblk=nblk),
        in_specs=[pl.BlockSpec(memory_space=pl.ANY), pl.BlockSpec(memory_space=pl.ANY)],
        out_specs=pl.BlockSpec(memory_space=pl.ANY),
        out_shape=jax.ShapeDtypeStruct((B, T, D), x.dtype),
        scratch_shapes=[
            pltpu.VMEM((2, P * (Q + 4) + 8, _LANES), jnp.uint32),
            pltpu.VMEM((len(plan.g_slot), 2 * D // _LANES, D // 2, _LANES), jnp.uint32),
            pltpu.VMEM((plan.n_in, 2, 2, Q, _LANES), jnp.float32),
            pltpu.VMEM((plan.n_out, 2 * Q, 2 * D), jnp.float32),
            pltpu.VMEM((2, P * (Q + 4), _LANES), jnp.uint32),
            pltpu.VMEM((K, D, 2 * D), w.dtype),
            pltpu.VMEM((2, _HALO + TM, D), x.dtype),
            pltpu.VMEM((2, TM, D), x.dtype),
            pltpu.SemaphoreType.DMA((_W_SLABS,)),
            pltpu.SemaphoreType.DMA((2, 2)),
            pltpu.SemaphoreType.DMA((2,)),
        ],
        compiler_params=pltpu.CompilerParams(vmem_limit_bytes=100 * 1024 * 1024),
    )(x, w)
```

```python
import functools
import math

import jax
import jax.numpy as jnp
import jax.experimental.pallas as pl
import jax.experimental.pallas.tpu as pltpu

_LEVELS = "WBBKK"
_MATERIALISE = (1, 2, 3)
_Q = 24
_HALO = 64
_HALO32 = _HALO // 2
_W_SLABS = 16
_W_DEPTH = 6
_LANES = 128


class _Node:
    def __init__(self, kind, parent, taps, nout, path):
        self.kind, self.parent, self.taps, self.nout, self.path = kind, parent, taps, nout, path
        self.depth = len(path)
        self.children = None

    def din(self, r):
        h = self.nout
        return {
            "K0": [(1, 2 * r), (-1, 2 * r + 1)], "Km": [(1, 2 * r + 1)], "K1": [(1, 2 * r + 2), (-1, 2 * r + 1)],
            "B0": [(1, r), (-1, h + r)], "Bm": [(1, h + r)], "B1": [(1, 2 * h + r), (-1, h + r)],
            "W0": [(1, r), (-1, 2 * h + r)], "W1": [(1, h + r), (1, 2 * h + r)],
            "W2": [(1, 2 * h + r), (-1, h + r)], "W3": [(1, 3 * h + r), (-1, h + r)],
        }[self.kind]


def _tap_sum(a, b, sign=1):
    return {**a, **{k: sign * v for k, v in b.items()}}


def _build_tree(ktaps, levels):
    nout = math.prod(3 if lv == "W" else 2 for lv in levels)
    root = _Node("root", None, [{k: 1} for k in range(ktaps)], nout, ())

    def split(n, rest):
        if not rest:
            return
        lv = rest[0]
        if lv == "K":
            h, lo, hi = n.nout // 2, n.taps[0::2], n.taps[1::2]
        else:
            h = n.nout // (3 if lv == "W" else 2)
            lo, hi = n.taps[:h], n.taps[h:]
        mix = lambda sign: [_tap_sum(a, hi[j], sign) if j < len(hi) else a for j, a in enumerate(lo)]
        if lv == "W":
            kids = [("W0", lo), ("W1", mix(1)), ("W2", mix(-1)), ("W3", hi)]
        else:
            kids = [(lv + "0", lo), (lv + "m", mix(1)), (lv + "1", hi)]
        n.children = [_Node(k, n, t, h, n.path + (i,)) for i, (k, t) in enumerate(kids)]
        for c in n.children:
            split(c, rest[1:])

    split(root, levels)
    return root


class _Plan:
    def __init__(self, ktaps, levels, materialise, q):
        self.root = _build_tree(ktaps, levels)
        self.P = self.root.nout
        self.materialise = materialise
        self.items = []
        self._arrays = 0
        self._output_network()
        self._input_network(q)

    def _new(self, n):
        self._arrays += n
        return list(range(self._arrays - n, self._arrays))

    def _solve(self, n, inits, sinks):
        if n.children is None:
            self.items.append(("leaf", n, inits[0], sinks[0]))
            return
        c0, cm, c1 = n.children
        half = n.nout // 2
        mids = self._new(half)
        self._solve(cm, [[] for _ in mids], [("store", m) for m in mids])
        i0, i1 = (range(half), range(half, n.nout)) if c0.kind == "B0" else (range(0, n.nout, 2), range(1, n.nout, 2))
        for c, idx in ((c0, i0), (c1, i1)):
            self._solve(c, [inits[i] + [m] for i, m in zip(idx, mids)], [sinks[i] for i in idx])

    def _output_network(self):
        w0, w1, w2, w3 = self.root.children
        h = self.P // 3
        m1, s = self._new(h), self._new(h)
        self._solve(w1, [[] for _ in m1], [("store", m) for m in m1])
        self._solve(w2, [[m] for m in m1], [("half", a) for a in s])
        head, n0 = self.items, len(self.items)
        self._solve(w0, [[a] for a in s], [("final", i) for i in range(h)])
        self._solve(w3, [[a] for a in s], [("final", 2 * h + i) for i in range(h)])
        combs = [("comb", None, (m1[i], s[i]), ("final", h + i)) for i in range(h)]
        rest = head[n0:]
        self.items = head[:n0]
        every = max(1, len(rest) // (h + 1))
        for i, it in enumerate(rest):
            self.items.append(it)
            if (i + 1) % every == 0 and combs:
                self.items.append(combs.pop(0))
        self.items += combs

    def _expr(self, n, r):
        return [(s * s2, src) for s, pr in n.din(r) for s2, src in self._resolve(n.parent, pr)]

    def _resolve(self, n, r):
        if n.parent is None:
            return [(1, ("x", r))]
        e = self._expr(n, r)
        if n.depth not in self.materialise or (len(e) == 1 and e[0][0] == 1):
            return e
        key = ("a", n.path, r)
        self.prep_expr[key] = e
        return [(1, key)]

    def _input_network(self, q):
        items, n = self.items, len(self.items)
        self.prep_expr, self.leaf_expr, deadline = {}, {}, {}
        for i, it in enumerate(items):
            if it[0] == "leaf" and it[1].taps:
                self.leaf_expr[it[1].path] = e = self._expr(it[1], 0)
                for _, src in e:
                    deadline.setdefault(src, i)
        cap = max(1, math.ceil(1.15 * len(self.prep_expr) / n))
        load, slot = {}, {}
        depth = lambda key: len(key[1])
        for d in sorted(set(map(depth, self.prep_expr)), reverse=True):
            for k in sorted((k for k in self.prep_expr if depth(k) == d), key=lambda k: -deadline[k]):
                s = max(deadline[k] - 1, 0)
                while s > 0 and load.get(s, 0) >= cap:
                    s -= 1
                slot[k] = s
                load[s] = load.get(s, 0) + 1
                for _, src in self.prep_expr[k]:
                    if src[0] == "a":
                        deadline[src] = min(deadline.get(src, n), s)
        before = [[] for _ in range(n)]
        for k in sorted(slot, key=lambda k: (slot[k], depth(k))):
            before[slot[k]].append(("prep", k))
        first_final = min(i for i, it in enumerate(items) if it[3][0] == "final")
        unstage = [("unstage", c, i) for i in range(q) for c in range(2)]
        for i, op in enumerate(unstage):
            before[3 + i * (first_final - 11) // len(unstage)].append(op)
        self.unstage = unstage
        self.ops = [("halo", c, 0) for c in range(2)] + [("stage", c, i) for i in range(q) for c in range(2)]
        body = [op for b, it in zip(before, items) for op in b + [it]]
        self.ops += body

        last_in, last_out = {}, {}
        for t, op in enumerate(body):
            if op[0] == "prep":
                last_in.update({src: t for _, src in self.prep_expr[op[1]] if src[0] == "a"})
            elif op[0] == "leaf":
                last_in.update({src: t for _, src in self.leaf_expr.get(op[1].path, ())})
            if op[0] in ("leaf", "comb"):
                last_out.update({a: t for a in op[2]})

        def allocate(defs, last):
            slots, free, pending, count, release = {}, [], [], 0, {}
            for k, t in last.items():
                release.setdefault(t, []).append(k)
            for t, k in enumerate(defs):
                if k is not None:
                    if not free:
                        free.append(count)
                        count += 1
                    slots[k] = free.pop(0)
                pending += [(t, r) for r in release.get(t, [])]
                while pending and pending[0][0] <= t - 2:
                    free.append(slots[pending.pop(0)[1]])
            return slots, max(count, 1)

        self.in_slot, self.n_in = allocate([op[1] if op[0] == "prep" else None for op in body], last_in)
        self.out_slot, self.n_out = allocate(
            [op[3][1] if op[0] in ("leaf", "comb") and op[3][0] != "final" else None for op in body], last_out)

        self.g_slot, self.g_raw = {}, {}
        for it in items:
            if it[0] == "leaf" and it[1].taps:
                (tap,) = it[1].taps
                if it[1].path[0] in (0, 3) and len(tap) == 1:
                    (self.g_raw[it[1].path],) = tap
                else:
                    self.g_slot[it[1].path] = len(self.g_slot)


def _pack(lo, hi):
    return pltpu.pack_elementwise([lo, hi], packed_dtype=jnp.bfloat16)


def _unpack(v):
    return pltpu.bitcast(v << 16, jnp.float32), pltpu.bitcast(v & jnp.uint32(0xFFFF0000), jnp.float32)


def _signed_sum(terms):
    pos = [v for s, v in terms if s > 0]
    neg = [v for s, v in terms if s < 0]
    parts = []
    while pos and neg:
        parts.append(pos.pop(0) - neg.pop(0))
    parts += pos
    while len(parts) > 1:
        parts = [parts[i] + parts[i + 1] if i + 1 < len(parts) else parts[i] for i in range(0, len(parts), 2)]
    acc = parts[0]
    for v in neg:
        acc = acc - v
    return acc


def _kernel(x_hbm, w_hbm, o_hbm, pm_ref, g_ref, a_ref, b_ref, po_ref, w_ref, x_buf, o_buf, w_sem, x_sem, o_sem,
            *, plan, nb, T, K, D, nblk):
    P, Q = plan.P, _Q
    QS = Q + 4
    TM = 2 * P * Q
    N = nb * nblk
    RW = D // _W_SLABS
    halves, ntiles = D // _LANES, 2 * D // _LANES
    lanes = lambda c: slice(c * _LANES, (c + 1) * _LANES)
    zero = jnp.int32(0)

    def row0(t):
        return pl.multiple_of(jnp.where(t > 0, T - (nblk - t) * TM, 0), 16)

    def x_copies(b, t, slot):
        t0 = row0(t)
        h0 = pl.multiple_of(jnp.maximum(t0 - _HALO, 0), 16)
        return (pltpu.make_async_copy(x_hbm.at[b, pl.ds(h0, _HALO), :], x_buf.at[slot, pl.ds(0, _HALO), :],
                                      x_sem.at[2 * slot]),
                pltpu.make_async_copy(x_hbm.at[b, pl.ds(t0, TM), :], x_buf.at[slot, pl.ds(_HALO, TM), :],
                                      x_sem.at[2 * slot + 1]))

    def o_copy(b, t, slot):
        return pltpu.make_async_copy(o_buf.at[slot], o_hbm.at[b, pl.ds(row0(t), TM), :], o_sem.at[slot])

    def w_copy(i):
        r = pl.ds(pl.multiple_of(i * RW, RW), RW)
        return pltpu.make_async_copy(w_hbm.at[:, r, :], w_ref.at[:, r, :], w_sem.at[i])

    def g_tap(n, load_tap, memo, j):
        key = (n.path, j)
        if key not in memo:
            f32 = lambda v: _unpack(v[1]) if v[0] == "w" else v[1:]
            k, par = n.kind, n.parent
            if k == "root":
                out = ("w", load_tap(j))
            elif k in ("K0", "K1", "B0", "B1", "W0", "W3"):
                jp = {"K0": 2 * j, "K1": 2 * j + 1, "B0": j, "W0": j, "B1": n.nout + j, "W3": n.nout + j}[k]
                out = g_tap(par, load_tap, memo, jp)
            else:
                j0, j1 = (2 * j, 2 * j + 1) if k == "Km" else (j, n.nout + j)
                out = g_tap(par, load_tap, memo, j0)
                if j1 < len(par.taps):
                    (l0, h0), (l1, h1) = f32(out), f32(g_tap(par, load_tap, memo, j1))
                    out = ("f", l0 - l1, h0 - h1) if k == "W2" else ("f", l0 + l1, h0 + h1)
                elif k[0] == "W":
                    out = ("f",) + tuple(f32(out))
            memo[key] = out
        return memo[key]

    def g_leaves(n):
        if n.children is None:
            return [n] if n.path in plan.g_slot else []
        order = (1, 2, 0, 3) if n.parent is None else (2, 0, 1)
        return [lf for i in order for lf in g_leaves(n.children[i])]

    def transform_slab(i, copy_next):
        w_copy(i).wait()
        if copy_next:
            w_copy(i + _W_DEPTH).start()
        r0 = pl.multiple_of(i * RW, 16)
        s0 = pl.multiple_of(i * (RW // 2), 8)
        for nt in range(ntiles):
            memo, top = {}, None
            for lf in g_leaves(plan.root):
                if lf.path[:2] != top:
                    top, memo = lf.path[:2], {}
                load_tap = lambda k: pltpu.bitcast(w_ref[k, pl.ds(r0, 16), lanes(nt)], jnp.uint32)
                v = g_tap(lf, load_tap, memo, 0)
                g_ref[plan.g_slot[lf.path], nt, pl.ds(s0, 8), :] = v[1] if v[0] == "w" else _pack(v[1], v[2])
        return 0

    off0 = _HALO32 - (K - 1) + (P - _HALO32)

    def load(src, c):
        if src[0] == "x":
            rho = src[1] + off0
            return _unpack(pm_ref[c, pl.ds((rho % P) * QS + rho // P, Q), :])
        sl = plan.in_slot[src]
        return a_ref[sl, c, 0], a_ref[sl, c, 1]

    def evaluate(e, c):
        vals = [(s, load(src, c)) for s, src in e]
        return _signed_sum([(s, v[0]) for s, v in vals]), _signed_sum([(s, v[1]) for s, v in vals])

    def sink(y, to):
        if to[0] == "final":
            tf = jnp.tanh(y[:, :D])
            o = (0.5 * (tf * jnp.tanh(0.5 * y[:, D:]) + tf)).astype(jnp.bfloat16)
            for c in range(halves):
                po_ref[c, pl.ds(to[1] * QS, Q), :] = pltpu.bitcast(o[:, lanes(c)], jnp.uint32)
        else:
            b_ref[plan.out_slot[to[1]]] = y if to[0] == "store" else 0.5 * y

    def emit(ops, keep_halo, slot):
        for op in ops:
            kind = op[0]
            if kind == "prep":
                sl = plan.in_slot[op[1]]
                for c in range(halves):
                    a_ref[sl, c, 0], a_ref[sl, c, 1] = evaluate(plan.prep_expr[op[1]], c)
            elif kind == "leaf":
                _, n, inits, to = op
                acc = None
                for a in inits:
                    v = b_ref[plan.out_slot[a]]
                    acc = v if acc is None else acc + v
                if n.taps:
                    lhs = jnp.concatenate(
                        [pltpu.bitcast(_pack(*evaluate(plan.leaf_expr[n.path], c)), jnp.bfloat16)
                         for c in range(halves)], axis=1)
                    if n.path in plan.g_raw:
                        rhs = w_ref[plan.g_raw[n.path]]
                    else:
                        rhs = jnp.concatenate([pltpu.bitcast(g_ref[plan.g_slot[n.path], nt], jnp.bfloat16)
                                               for nt in range(ntiles)], axis=1)
                    prod = jnp.dot(lhs, rhs, preferred_element_type=jnp.float32)
                    acc = prod if acc is None else acc + prod
                sink(acc, to)
            elif kind == "comb":
                _, _, (m1, s), to = op
                sink(b_ref[plan.out_slot[m1]] - b_ref[plan.out_slot[s]], to)
            elif kind == "halo":
                c = op[1]
                halo = pltpu.bitcast(x_buf[slot, pl.ds(0, _HALO), lanes(c)], jnp.uint32)
                pm_ref[c, pl.ds((P - _HALO32) * QS, _HALO32, stride=QS), :] = jnp.where(
                    keep_halo, halo, jnp.zeros_like(halo))
            elif kind == "stage":
                _, c, i = op
                pm_ref[c, pl.ds(i + 1, P, stride=QS), :] = pltpu.bitcast(
                    x_buf[slot, pl.ds(_HALO + 2 * P * i, 2 * P), lanes(c)], jnp.uint32)
            else:
                _, c, i = op
                o_buf[slot, pl.ds(2 * P * i, 2 * P), lanes(c)] = pltpu.bitcast(
                    po_ref[c, pl.ds(i, P, stride=QS), :], jnp.bfloat16)

    for i in range(_W_DEPTH):
        w_copy(i).start()
    po_ref[...] = jnp.zeros(po_ref.shape, po_ref.dtype)
    jax.lax.fori_loop(0, _W_SLABS - _W_DEPTH, lambda i, _: transform_slab(i, True), 0)
    for cp in x_copies(zero, zero, 0):
        cp.start()
    jax.lax.fori_loop(_W_SLABS - _W_DEPTH, _W_SLABS, lambda i, _: transform_slab(i, False), 0)

    def block(n, carry):
        b, t, pb, pt = carry
        slot = n & 1
        wrap, last = t == nblk - 1, n == N - 1
        nxt_b = jnp.where(last, b, jnp.where(wrap, b + 1, b))
        nxt_t = jnp.where(last, t, jnp.where(wrap, 0, t + 1))
        for cp in x_copies(b, t, slot):
            cp.wait()
        for cp in x_copies(nxt_b, nxt_t, 1 - slot):
            cp.start()
        emit(plan.ops, t > 0, slot)
        pl.when(n >= 2)(lambda: o_copy(pb, pt, 1 - slot).wait())
        pl.when(n >= 1)(lambda: o_copy(pb, pt, slot).start())
        return nxt_b, nxt_t, b, t

    b, t, pb, pt = jax.lax.fori_loop(0, N, block, (zero, zero, zero, zero))
    slot = N & 1
    emit(plan.unstage, False, slot)
    o_copy(pb, pt, slot).start()
    for cp in x_copies(b, t, slot):
        cp.wait()
    o_copy(pb, pt, 1 - slot).wait()
    o_copy(pb, pt, slot).wait()


@jax.jit
def pallas_standalone__autoregressive_conv_wavernn__speech_kernel(x: jax.Array, w: jax.Array):
    B, T, D = x.shape
    K = w.shape[0]
    plan = _Plan(K, _LEVELS, _MATERIALISE, _Q)
    P, Q = plan.P, _Q
    TM = 2 * P * Q
    nblk = pl.cdiv(T, TM)
    assert D == 2 * _LANES and K - 1 <= _HALO32 <= P and D == 16 * _W_SLABS
    assert nblk >= 3 and T % 16 == 0 and T - (nblk - 1) * TM >= _HALO
    return pl.pallas_call(
        functools.partial(_kernel, plan=plan, nb=B, T=T, K=K, D=D, nblk=nblk),
        in_specs=[pl.BlockSpec(memory_space=pl.ANY), pl.BlockSpec(memory_space=pl.ANY)],
        out_specs=pl.BlockSpec(memory_space=pl.ANY),
        out_shape=jax.ShapeDtypeStruct((B, T, D), x.dtype),
        scratch_shapes=[
            pltpu.VMEM((2, P * (Q + 4) + 8, _LANES), jnp.uint32),
            pltpu.VMEM((len(plan.g_slot), 2 * D // _LANES, D // 2, _LANES), jnp.uint32),
            pltpu.VMEM((plan.n_in, 2, 2, Q, _LANES), jnp.float32),
            pltpu.VMEM((plan.n_out, 2 * Q, 2 * D), jnp.float32),
            pltpu.VMEM((2, P * (Q + 4), _LANES), jnp.uint32),
            pltpu.VMEM((K, D, 2 * D), w.dtype),
            pltpu.VMEM((2, _HALO + TM, D), x.dtype),
            pltpu.VMEM((2, TM, D), x.dtype),
            pltpu.SemaphoreType.DMA((_W_SLABS,)),
            pltpu.SemaphoreType.DMA((4,)),
            pltpu.SemaphoreType.DMA((2,)),
        ],
        compiler_params=pltpu.CompilerParams(vmem_limit_bytes=100 * 1024 * 1024),
    )(x, w)
```
